```python
import jax
import jax.numpy as jnp

def _softmax(x, axis=-1):
    return jax.nn.softmax(x, axis=axis)
def _gelu(x):
    return jax.nn.gelu(x, approximate=True)
def _silu(x):
    return jax.nn.silu(x)
def _sigmoid(x):
    return jax.nn.sigmoid(x)
def _layernorm(x, axis=-1, eps=1e-5):
    m = jnp.mean(x, axis=axis, keepdims=True)
    v = jnp.var(x, axis=axis, keepdims=True)
    return (x - m) / jnp.sqrt(v + eps)
def _scatter_add(tgt, idx, src, axis=0):
    return tgt.at[idx].add(src)
def _segment_sum(src, seg, n):
    return jax.ops.segment_sum(src, seg, n)
class _Rng:
    def __init__(self, key):
        self._k = key
    def _next(self):
        self._k, sub = jax.random.split(self._k)
        return sub
    def normal(self, shape):
        return jax.random.normal(self._next(), shape, dtype=jnp.bfloat16)
    def randint(self, lo, hi, shape):
        return jax.random.randint(self._next(), shape, lo, hi, dtype=jnp.int32)
    def uniform(self, shape, lo=0.0, hi=1.0):
        return jax.random.uniform(self._next(), shape, jnp.bfloat16, lo, hi)
    def permutation(self, n):
        return jax.random.permutation(self._next(), n)


kernel_name = 'recurrent_scan__mha_block_cached__moe_arch_mod__prompt'

def setup_inputs():
    _rng = _Rng(jax.random.key(int.from_bytes(__import__("os").urandom(4), "little")))
    _w = (lambda a: (lambda t: t.astype(jnp.bfloat16) if jnp.issubdtype(t.dtype, jnp.floating) else t)(jnp.asarray(a)))
    def _A_setup():
        B, Sq, D = 1, 2048, 640
        H, Sk, Dh = 32, 2048, 128
        return {
            "x": _w((lambda *s: _rng.normal(s) * 0.05)(B, Sq, D)),
            "k_cache": _w((lambda *s: _rng.normal(s) * 0.05)(B, H, Sk, Dh)),
            "v_cache": _w((lambda *s: _rng.normal(s) * 0.05)(B, H, Sk, Dh)),
            "wq": _w((lambda *s: _rng.normal(s) * 0.05)(D, H * Dh) * (D ** -0.5)),
            "wo": _w((lambda *s: _rng.normal(s) * 0.05)(H * Dh, D) * ((H * Dh) ** -0.5)),
        }
    _A_in = _A_setup()

    def _B_setup():
        B, S, D, F, C = 1, 2048, 640, 1728, 8
        return {
            "x": _w((lambda *s: _rng.normal(s) * 0.05)(B, S, D)),
            "w_r": _w((lambda *s: _rng.normal(s) * 0.05)(D)),
            "w_gate": _w((lambda *s: _rng.normal(s) * 0.05)(D, F)),
            "w_up": _w((lambda *s: _rng.normal(s) * 0.05)(D, F)),
            "w_down": _w((lambda *s: _rng.normal(s) * 0.05)(F, D)),
        }
    _B_in = _B_setup()

    return {
        "A_x": _A_in["x"],
        "A_k_cache": _A_in["k_cache"],
        "A_v_cache": _A_in["v_cache"],
        "A_wq": _A_in["wq"],
        "A_wo": _A_in["wo"],
        "B_x": _B_in["x"],
        "B_w_r": _B_in["w_r"],
        "B_w_gate": _B_in["w_gate"],
        "B_w_up": _B_in["w_up"],
        "B_w_down": _B_in["w_down"],
    }

def reference(A_x, A_k_cache, A_v_cache, A_wq, A_wo, B_x, B_w_r, B_w_gate, B_w_up, B_w_down):
    def _A_ref(x, k_cache, v_cache, wq, wo):
        B, Sq, D = x.shape
        H, Dh = 32, 128
        q = (lambda x, *d: x.transpose(*d))((x @ wq).reshape(B, Sq, H, Dh), 0, 2, 1, 3)
        scores = jnp.einsum("bhqd,bhkd->bhqk", q, k_cache) * (Dh ** -0.5)
        p = _softmax(scores, axis=-1)
        o = jnp.einsum("bhqk,bhkd->bhqd", p, v_cache)
        return (lambda x, *d: x.transpose(*d))(o, 0, 2, 1, 3).reshape(B, Sq, H * Dh) @ wo

    def _B_ref(x, w_r, w_gate, w_up, w_down):
        B, S, D = x.shape
        C = 8
        r = x @ w_r
        idx = jnp.argsort(-r, axis=-1)[:, :C]
        idx_e = jnp.repeat(idx.reshape(B, C, 1), D, axis=2)
        x_sel = jnp.take_along_axis(x, idx_e, axis=1)
        g = _silu(x_sel @ w_gate)
        u = x_sel @ w_up
        y = (g * u) @ w_down
        r_sel = _sigmoid(jnp.take_along_axis(r, idx, axis=1))
        y = y * r_sel.reshape(B, C, 1)
        b_off = (jnp.arange(B) * S).reshape(B, 1)
        flat_idx = (idx + b_off).reshape(B * C)
        zero = (x * 0.0).reshape(B * S, D)
        upd = _scatter_add(zero, flat_idx, y.reshape(B * C, D), axis=0)
        return x + upd.reshape(B, S, D)

    x = A_x
    xn = _layernorm(x, axis=-1)
    s = _A_ref(xn, A_k_cache, A_v_cache, A_wq, A_wo)
    g = _silu(_B_ref(xn, B_w_r, B_w_gate, B_w_up, B_w_down))
    return x + s * g
```

```python
import functools
import jax
import jax.numpy as jnp
from jax import lax
import jax.experimental.pallas as pl
import jax.experimental.pallas.tpu as pltpu

S, D, HH, DH, F, C = 2048, 640, 32, 128, 1728, 8
LOG2E = 1.4426950408889634
NT = (((1,), (1,)), ((), ()))
f32 = jnp.float32
bf16 = jnp.bfloat16


def _rb(a):
    return a.astype(bf16).astype(f32)


def _gate(m, tok):
    return jnp.maximum(m, jnp.minimum(m, tok))


def _sigmoid(x):
    return 0.5 * jnp.tanh(0.5 * x) + 0.5


def make(G=256, KC=512, skew=1, lag=2, qpos=1, opos=1, lnahead=3, xsplit=(1, 3, 4), modpos=1, qk_first=True,
         variants='FML', nbuf=4, fmode='pre', lmode='post', H=32, nodma=False, skip='', smode='dyn'):
    ng = S // G
    nk = S // KC
    ahead = nk + skew
    nx = len(xsplit)
    xoff = [sum(xsplit[:i]) for i in range(nx)]

    def kernel(x_hbm, k_hbm, v_hbm, wq_hbm, wo_hbm, wr_ref, wg_hbm, wu_hbm, wd_hbm, o_hbm,
               x_ref, kbuf, vbuf, wqbuf, wobuf, wg_ref, wu_ref, wd_ref, ob_ref,
               xn_ref, z_ref, acc_ref, r_ref, vt_ref,
               m_c, l_c, o_c, q_c,
               xsem, ksem, vsem, wqsem, wosem, fsem, osem, *s_refs):

        def x_cp(i):
            rows = pl.ds(xoff[i] * G, xsplit[i] * G)
            return pltpu.make_async_copy(x_hbm.at[rows, :], x_ref.at[rows, :], xsem.at[i])

        def k_cp(h, slot):
            return pltpu.make_async_copy(k_hbm.at[h], kbuf.at[slot], ksem.at[slot])

        def v_cp(h, slot):
            return pltpu.make_async_copy(v_hbm.at[h], vbuf.at[slot], vsem.at[slot])

        def wq_cp(h, slot):
            col = h * DH if isinstance(h, int) else pl.multiple_of(h * DH, DH)
            return pltpu.make_async_copy(wq_hbm.at[:, pl.ds(col, DH)], wqbuf.at[slot], wqsem.at[slot])

        def wo_cp(h, slot):
            row = h * DH if isinstance(h, int) else pl.multiple_of(h * DH, DH)
            return pltpu.make_async_copy(wo_hbm.at[pl.ds(row, DH), :], wobuf.at[slot], wosem.at[slot])

        def f_cp(i):
            src = (wg_hbm, wu_hbm, wd_hbm)[i]
            dst = (wg_ref, wu_ref, wd_ref)[i]
            return pltpu.make_async_copy(src, dst, fsem.at[i])

        def o_cp(c):
            rows = pl.ds(c * G, G)
            return pltpu.make_async_copy(ob_ref.at[rows, :], o_hbm.at[rows, :], osem.at[c])

        def step(h, first, last, mode='full'):
            if isinstance(h, int):
                s2, s3, s3p, s3n = h % 2, h % 3, (h - 1) % 3, (h + 1) % 3
            else:
                s2 = lax.rem(h, 2)
                s3 = lax.rem(h, 3)
                s3p = lax.rem(h + 2, 3)
                s3n = lax.rem(h + 1, 3)
            k_ref = kbuf.at[s2]
            v_ref = vbuf.at[s2]
            zero = 0 if isinstance(h, int) else jnp.minimum(h, 0)

            def srow(j):
                return pl.ds(j * KC, KC) if isinstance(h, int) else pl.ds(pl.multiple_of(zero + j * KC, KC), KC)

            def grow(c):
                return pl.ds((c % ng) * G, G)

            qs, maccs, ms, laccs, oaccs = {}, {}, {}, {}, {}
            hist = []
            lastm = [None]
            xwaited = set()

            def ln(c):
                for i in range(nx):
                    if xoff[i] <= c < xoff[i] + xsplit[i] and i not in xwaited:
                        x_cp(i).wait()
                        xwaited.add(i)
                x = x_ref[grow(c), :].astype(f32)
                mean = jnp.sum(x, axis=-1, keepdims=True) * (1.0 / D)
                xc = x - mean
                var = jnp.sum(xc * xc, axis=-1, keepdims=True) * (1.0 / D)
                den = _rb(jnp.sqrt(_rb(_rb(var) + _rb(f32(1e-5)))))
                xnb = (_rb(x - _rb(mean)) * (1.0 / den)).astype(bf16)
                xn_ref[grow(c), :] = xnb
                z_ref[grow(c), :] = xnb.astype(f32)
                wr8 = jnp.broadcast_to(wr_ref[...], (16, D))
                rt = lax.dot_general(wr8, xnb, NT, preferred_element_type=f32)
                r_ref[c:c + 1, :] = rt[0:1, :]

            def qproj(c):
                w = wqbuf[s3] if c < ng else wqbuf[s3n]
                q = jnp.dot(xn_ref[grow(c), :], w, preferred_element_type=f32)
                qs[c] = (q * (DH ** -0.5 * LOG2E)).astype(bf16)

            def qk(c, j):
                st = lax.dot_general(k_ref[j * KC:(j + 1) * KC, :], qs[c], NT, preferred_element_type=f32)
                if smode in ('dyn', 'dynst'):
                    s_refs[c % nbuf][srow(j), :] = st
                else:
                    s_refs[c % nbuf][j * KC:(j + 1) * KC, :] = st
                mm = jnp.max(st.reshape(KC // 8, 8, G), axis=0)
                maccs[c] = mm if j == 0 else jnp.maximum(maccs[c], mm)
                lastm[0] = maccs[c]

            def vtr(j):
                if 'v' in skip:
                    return
                vt_ref[:, j * KC:(j + 1) * KC] = v_ref[j * KC:(j + 1) * KC, :].T

            def pv(c, j):
                if j == 0:
                    ms[c] = jnp.broadcast_to(jnp.max(maccs[c], axis=0, keepdims=True), (8, G))
                m = ms[c]
                if lag and len(hist) >= lag:
                    for tok in hist[len(hist) - lag]:
                        m = _gate(m, tok)
                if smode == 'dyn':
                    sv = s_refs[c % nbuf][srow(j), :]
                elif smode == 'static':
                    sv = s_refs[c % nbuf][j * KC:(j + 1) * KC, :]
                elif smode == 'halves':
                    sv = jnp.concatenate([s_refs[c % nbuf][j * KC:(j + 1) * KC, t * 128:(t + 1) * 128] for t in range(G // 128)], axis=1)
                elif smode == 'dynld':
                    sv = s_refs[c % nbuf][srow(j), :]
                elif smode == 'dynst':
                    sv = s_refs[c % nbuf][j * KC:(j + 1) * KC, :]
                p = sv.reshape(KC // 8, 8, G) - m[None]
                if 'e' not in skip:
                    p = jnp.exp2(p)
                ll = jnp.sum(p, axis=0)
                laccs[c] = ll if j == 0 else laccs[c] + ll
                oo = jnp.dot(vt_ref[:, j * KC:(j + 1) * KC], p.reshape(KC, G).astype(bf16),
                             preferred_element_type=f32)
                oaccs[c] = oo if j == 0 else oaccs[c] + oo
                hist.append([t for t in (lastm[0], laccs[c], oaccs[c][DH - 8:, :]) if t is not None])

            def oproj(c):
                l = jnp.sum(laccs[c], axis=0, keepdims=True)
                if 't' in skip:
                    o = (oaccs[c] * (1.0 / l)).astype(bf16)
                    o = jnp.concatenate([o[:, :128], o[:, 128:]], axis=0)
                else:
                    o = (oaccs[c] * (1.0 / l)).T.astype(bf16)
                w = wobuf[s3] if c >= 0 else wobuf[s3p]
                y = jnp.dot(o, w, preferred_element_type=f32)
                if first:
                    acc_ref[grow(c), :] = y
                elif last and c >= 0:
                    s = acc_ref[grow(c), :] + y
                    z = z_ref[grow(c), :]
                    ob_ref[grow(c), :] = (x_ref[grow(c), :].astype(f32) + s * (z * _sigmoid(z))).astype(bf16)
                    o_cp(c).start()
                else:
                    acc_ref[grow(c), :] += y

            def mod():
                r = _rb(r_ref[...])
                r = jnp.where(r != r, -jnp.inf, r)
                ids = (lax.broadcasted_iota(jnp.int32, (ng, G), 0) * G
                       + lax.broadcasted_iota(jnp.int32, (ng, G), 1))
                taken = jnp.zeros((ng, G), jnp.bool_)
                rid = lax.broadcasted_iota(jnp.int32, (C, 1), 0)
                rsel = jnp.zeros((C, 1), f32)
                idxs, rows = [], []
                for j in range(C):
                    cand = jnp.where(taken, -jnp.inf, r)
                    mx = jnp.max(cand, keepdims=True)
                    hit = jnp.logical_and(cand == mx, jnp.logical_not(taken))
                    am = jnp.min(jnp.where(hit, ids, S - 1))
                    taken = jnp.logical_or(taken, ids == am)
                    rsel = jnp.where(rid == j, mx, rsel)
                    idxs.append(am)
                    rows.append(z_ref[pl.ds(am, 1), :])
                xs = jnp.concatenate(rows, axis=0)
                xsb = xs.astype(bf16)
                for i in range(3):
                    f_cp(i).wait()
                a = lax.dot_general(xsb, wg_ref[...], NT, preferred_element_type=f32)
                u = lax.dot_general(xsb, wu_ref[...], NT, preferred_element_type=f32)
                hh = (a * _sigmoid(a) * u).astype(bf16)
                y = jnp.dot(hh, wd_ref[...], preferred_element_type=f32)
                zz = xs + y * _sigmoid(rsel)
                for j in range(C):
                    z_ref[pl.ds(idxs[j], 1), :] = zz[j:j + 1, :]

            pos0 = -ahead
            cpart = pos0 // nk
            if first or mode == 'pre':
                x_cp(0).start()
                wq_cp(0, 0).start()
                k_cp(0, 0).start()
                for i in range(1, nx):
                    x_cp(i).start()
                v_cp(0, 0).start()
                wq_cp(1, 1).start()
                wo_cp(0, 0).start()
                ln(0)
                wq_cp(0, 0).wait()
                qproj(0)
            if mode == 'pre':
                for i in range(3):
                    f_cp(i).start()
                q_c[...] = qs[0]
                for c in range(1, ng):
                    ln(c)
                for c in range(cpart, 0):
                    s_refs[c % nbuf][...] = jnp.zeros((S, G), f32)
                m_c[...] = jnp.zeros(m_c.shape, f32)
                l_c[...] = jnp.ones(l_c.shape, f32)
                o_c[...] = jnp.zeros(o_c.shape, f32)
                vt_ref[...] = jnp.zeros(vt_ref.shape, bf16)
                wobuf[2] = jnp.zeros((DH, D), bf16)
                acc_ref[...] = jnp.zeros((S, D), f32)
                return
            if mode == 'full' and nodma:
                @pl.when(h == 0)
                def _():
                    k_cp(0, 0).wait()
                    v_cp(0, 0).wait()
                    wo_cp(0, 0).wait()
                    wq_cp(1, 1).wait()
            elif mode == 'full':
                dyn = not isinstance(h, int)
                k_cp(h, s2).wait()
                v_cp(h, s2).wait()
                wo_cp(h, s3).wait()
                if not last:
                    if dyn and lmode == 'post':
                        @pl.when(h + 1 < H)
                        def _():
                            wq_cp(h + 1, s3n).wait()
                            k_cp(h + 1, 1 - s2).start()
                            v_cp(h + 1, 1 - s2).start()
                            wo_cp(h + 1, s3n).start()
                    else:
                        wq_cp(h + 1, s3n).wait()
                        k_cp(h + 1, 1 - s2).start()
                        v_cp(h + 1, 1 - s2).start()
                        wo_cp(h + 1, s3n).start()
                    if first:
                        wq_cp(2, 2).start()
                        for i in range(3):
                            f_cp(i).start()
                    else:
                        @pl.when(h + 2 < H)
                        def _():
                            wq_cp(h + 2, s3p).start()

            if not first:
                qs[0] = q_c[...]
                for c in range(cpart, 0):
                    if c * nk < pos0:
                        ms[c] = m_c[c - cpart]
                        laccs[c] = l_c[0]
                        oaccs[c] = o_c[0]
                    else:
                        maccs[c] = m_c[c - cpart]
                if pos0 % nk <= opos:
                    laccs[cpart - 1] = l_c[1]
                    oaccs[cpart - 1] = o_c[1]
            else:
                for c in range(ng - 3, ng):
                    acc_ref[grow(c), :] = jnp.zeros((G, D), f32)

            if mode == 'post':
                mod()
                def fin(c):
                    z = z_ref[grow(c), :]
                    ob_ref[grow(c), :] = (x_ref[grow(c), :].astype(f32) + acc_ref[grow(c), :] * (z * _sigmoid(z))).astype(bf16)
                    o_cp(c % ng).start()
                todo = list(range(0, ng + (cpart - 1 if pos0 % nk <= opos else cpart)))
                for pos in range(pos0, 0):
                    c, j = pos // nk, pos % nk
                    pv(c, j)
                    if j == opos:
                        oproj(c - 1)
                        fin(c - 1)
                    if todo:
                        fin(todo.pop(0))
                for c in todo:
                    fin(c)
                oproj(-1)
                fin(-1)
                for c in range(ng):
                    o_cp(c).wait()
                return

            lndone = 1
            end = ng * nk if last else ng * nk - ahead
            for pos in range(pos0, end):
                c, j = pos // nk, pos % nk
                qi = pos + ahead

                def do_qk():
                    if qi < ng * nk:
                        qk(qi // nk, qi % nk)

                def do_pv():
                    if not (first and c < 0):
                        pv(c, j)

                if qk_first:
                    do_qk(); do_pv()
                else:
                    do_pv(); do_qk()
                if c == -1:
                    vtr(j)
                if first and lndone < ng and pos + lnahead >= (lndone - 2) * nk + qpos:
                    ln(lndone)
                    lndone += 1
                if last and pos == pos0 + modpos:
                    mod()
                if j == opos and not (first and c - 1 < 0):
                    oproj(c - 1)
                if j == qpos and c + 2 >= 1 and (c + 2 < ng or (c + 2 == ng and not last)):
                    qproj(c + 2)

            if last:
                oproj(ng - 1)
                for c in range(ng):
                    o_cp(c).wait()
            else:
                q_c[...] = qs[ng]
                for c in range(cpart, 0):
                    if c * nk < pos0:
                        m_c[c - cpart] = ms[c + ng]
                        l_c[0] = laccs[c + ng]
                        o_c[0] = oaccs[c + ng]
                    else:
                        m_c[c - cpart] = maccs[c + ng]
                if pos0 % nk <= opos:
                    l_c[1] = laccs[cpart - 1 + ng]
                    o_c[1] = oaccs[cpart - 1 + ng]

        step(0, False, False, 'pre')

        def mid(h, carry):
            step(h, False, False)
            return carry

        lax.fori_loop(0, H, mid, 0)
        step(H, False, False, 'post')

    @jax.jit
    def fn(A_x, A_k_cache, A_v_cache, A_wq, A_wo, B_x, B_w_r, B_w_gate, B_w_up, B_w_down):
        x = A_x.reshape(S, D)
        k = A_k_cache.reshape(HH, S, DH)
        v = A_v_cache.reshape(HH, S, DH)
        wr = B_w_r.reshape(1, D)
        hbm = pl.BlockSpec(memory_space=pl.ANY)
        V = pltpu.VMEM
        out = pl.pallas_call(
            kernel,
            in_specs=[hbm, hbm, hbm, hbm, hbm, pl.BlockSpec(memory_space=pltpu.VMEM), hbm, hbm, hbm],
            out_specs=hbm,
            out_shape=jax.ShapeDtypeStruct((S, D), bf16),
            scratch_shapes=[
                V((S, D), bf16), V((2, S, DH), bf16), V((2, S, DH), bf16), V((3, D, DH), bf16), V((3, DH, D), bf16),
                V((F, D), bf16), V((F, D), bf16), V((F, D), bf16), V((S, D), bf16),
                V((S, D), bf16), V((S, D), f32), V((S, D), f32), V((ng, G), f32), V((DH, S), bf16),
                V((2, 8, G), f32), V((2, 8, G), f32), V((2, DH, G), f32), V((G, DH), bf16),
                pltpu.SemaphoreType.DMA((nx,)), pltpu.SemaphoreType.DMA((2,)), pltpu.SemaphoreType.DMA((2,)),
                pltpu.SemaphoreType.DMA((3,)), pltpu.SemaphoreType.DMA((3,)), pltpu.SemaphoreType.DMA((3,)),
                pltpu.SemaphoreType.DMA((ng,)),
            ] + [V((S, G), f32)] * nbuf,
            compiler_params=pltpu.CompilerParams(vmem_limit_bytes=100 * 1024 * 1024),
        )(x, k, v, A_wq, A_wo, wr, B_w_gate.T, B_w_up.T, B_w_down)
        return out.reshape(1, S, D)

    return fn


_impl = make(**{'smode':'dynst'})


@jax.jit
def pallas_recurrent_scan__mha_block_cached__moe_arch_mod__prompt_kernel(A_x, A_k_cache, A_v_cache, A_wq, A_wo, B_x, B_w_r, B_w_gate, B_w_up, B_w_down):
    return _impl(A_x, A_k_cache, A_v_cache, A_wq, A_wo, B_x, B_w_r, B_w_gate, B_w_up, B_w_down)
```

```python
import jax
import jax.numpy as jnp
from jax import lax
import jax.experimental.pallas as pl
import jax.experimental.pallas.tpu as pltpu

S, D, HH, DH, F, C = 2048, 640, 32, 128, 1728, 8
LOG2E = 1.4426950408889634
NT = (((1,), (1,)), ((), ()))
f32 = jnp.float32
bf16 = jnp.bfloat16
u32 = jnp.uint32


def _rb(a):
    return a.astype(bf16).astype(f32)


def _gate(m, tok):
    return jnp.maximum(m, jnp.minimum(m, tok))


def _sigmoid(x):
    return 0.5 * jnp.tanh(0.5 * x) + 0.5


def _recip(d):
    r = pl.reciprocal(d, approx=True)
    r = r + r * (1.0 - d * r)
    return r + r * (1.0 - d * r)


def _pk(a):
    return pltpu.bitcast(a, u32)


def _upk(a):
    return pltpu.bitcast(a, bf16)


def make(G=256, KC=512, skew=1, lag=2, qpos=1, opos=1, nbuf=4, H=32, gates='mlo', B=12,
         lnsub=4, modpos=4, finlag=8, finsub=2, parts='PMQ', lntok=1, fintok=0, rb=16,
         w5=-1, w6=6, lastsub=4):
    ng = S // G
    nk = S // KC
    W = ng * nk
    ahead = nk + skew
    xsplit = (1, 1, 1, ng - 3)
    nx = len(xsplit)
    xoff = [sum(xsplit[:i]) for i in range(nx)]
    LR = G // lnsub

    p_qproj = lambda c: (c - 2) * nk + qpos
    p_qk = lambda c, j: c * nk + j - ahead
    p_pv = lambda c, j: c * nk + j
    p_op = lambda c: (c + 1) * nk + opos
    rng = range(-2, 2 * ng + 2)
    live_q = [c for c in rng if p_qproj(c) < B <= p_qk(c, nk - 1)]
    live_mx = [c for c in rng if p_qk(c, 0) < B <= p_pv(c, 0)]
    live_m = [c for c in rng if p_pv(c, 0) < B <= p_pv(c, nk - 1)]
    live_o = [c for c in rng if p_pv(c, 0) < B <= p_op(c)]

    def kernel(x_hbm, k_hbm, v_hbm, wq_hbm, wo_hbm, wr_ref, wg_hbm, wu_hbm, wd_hbm, o_hbm,
               zero_ref, x_ref, kbuf, vbuf, wqbuf, wobuf, wg_ref, wu_ref, wd_ref,
               xn_ref, z_ref, acc_ref, r_ref, kw_ref, vt_ref, wqw_ref, wow_ref,
               m_c, l_c, o_c, q_c,
               xsem, ksem, vsem, wqsem, wosem, fsem, osem, *rest):
        s_refs, ob_refs = rest[:nbuf], rest[nbuf:]

        def x_cp(i):
            rows = pl.ds(xoff[i] * G, xsplit[i] * G)
            return pltpu.make_async_copy(x_hbm.at[rows, :], x_ref.at[rows, :], xsem.at[i])

        def slot(h):
            return h % 3 if isinstance(h, int) else lax.rem(h, 3)

        def k_cp(h):
            return pltpu.make_async_copy(k_hbm.at[h], kbuf.at[slot(h)], ksem.at[slot(h)])

        def v_cp(h):
            return pltpu.make_async_copy(v_hbm.at[h], vbuf.at[slot(h)], vsem.at[slot(h)])

        def wq_cp(h):
            col = h * DH if isinstance(h, int) else pl.multiple_of(h * DH, DH)
            return pltpu.make_async_copy(wq_hbm.at[:, pl.ds(col, DH)], wqbuf.at[slot(h)], wqsem.at[slot(h)])

        def wo_cp(h):
            row = h * DH if isinstance(h, int) else pl.multiple_of(h * DH, DH)
            return pltpu.make_async_copy(wo_hbm.at[pl.ds(row, DH), :], wobuf.at[slot(h)], wosem.at[slot(h)])

        def f_cp(i):
            src = (wg_hbm, wu_hbm, wd_hbm)[i]
            dst = (wg_ref, wu_ref, wd_ref)[i]
            return pltpu.make_async_copy(src, dst, fsem.at[i])

        def o_cp(c, i=0, nsub=1):
            n = G // nsub
            return pltpu.make_async_copy(ob_refs[c].at[i * n:(i + 1) * n, :], o_hbm.at[pl.ds(c * G + i * n, n), :],
                                         osem.at[c + i])

        def grow(c):
            return pl.ds((c % ng) * G, G)

        def hrow(c):
            return pl.ds((c % ng) * (G // 2), G // 2)

        def segment(h, mode, zero):
            pre, post = mode == 'pre', mode == 'post'
            qs, maccs, ms, laccs, oaccs = {}, {}, {}, {}, {}
            hist = []
            lastm = [None]
            extra = []

            def done_token(ref, lagn):
                n = 16 if ref.dtype == bf16 else 8
                row = pl.ds(pl.multiple_of(zero + (ref.shape[0] - n), n), n)
                t = pltpu.bitcast(ref[row, 0:128], f32)
                extra.append((len(hist) + lagn, jnp.concatenate([t] * (G // 128), axis=1)))

            lane = lax.broadcasted_iota(jnp.int32, (8, 128), 1)
            racc = [jnp.zeros((8, 128), f32) for _ in range(S // 1024)]

            lnst = {}

            def ln_a(t):
                xs = []
                for r in range(t * LR, (t + 1) * LR, 16):
                    x16 = x_ref[r:r + 16, :].astype(f32)
                    xs += [x16[:8], x16[8:]]
                means = [jnp.sum(x, axis=-1, keepdims=True) * (1.0 / D) for x in xs]
                lnst[t] = dict(xs=xs, means=means)
                return means[-1]

            def ln_b(t):
                st = lnst[t]
                ssq = jnp.zeros((8, 128), f32)
                for k, (x, mean) in enumerate(zip(st['xs'], st['means'])):
                    xc = x - mean
                    ssq = jnp.where(lane == k, jnp.sum(xc * xc, axis=-1, keepdims=True), ssq)
                st['inv'] = 1.0 / _rb(jnp.sqrt(_rb(_rb(ssq * (1.0 / D)) + _rb(f32(1e-5)))))
                return st['inv']

            def ln_b2(t):
                st = lnst[t]
                st['invs'] = [jnp.sum(jnp.where(lane == k, st['inv'], 0.0), axis=-1, keepdims=True)
                              for k in range(LR // 8)]
                return st['invs'][-1]

            def ln_c(t):
                st = lnst[t]
                wr = jnp.broadcast_to(wr_ref[...].astype(f32), (8, D))
                for k in range(0, LR // 8, 2):
                    xn = jnp.concatenate([_rb(st['xs'][kk] - _rb(st['means'][kk])) * st['invs'][kk]
                                          for kk in (k, k + 1)], axis=0)
                    xnb = xn.astype(bf16)
                    r = t * LR + k * 8
                    xn_ref[r // 2:r // 2 + 8, :] = _pk(xnb)
                    z_ref[r // 2:r // 2 + 8, :] = _pk(xnb)
                    xr = xnb.astype(f32)
                    for kk in (0, 1):
                        rg = r // 8 + kk
                        rr = jnp.sum(xr[kk * 8:kk * 8 + 8] * wr, axis=-1, keepdims=True)
                        racc[rg // 128] = jnp.where(lane == rg % 128, rr, racc[rg // 128])
                del lnst[t]
                if (t + 1) % lnsub == 0:
                    lndone.add(t // lnsub)
                return racc[(t * LR) // 1024]

            lnstage = {}

            def tick(t, tok=True):
                toks = []
                for p in sorted(lnstage):
                    toks.append((ln_b, ln_b2, ln_c)[lnstage[p]](p))
                    lnstage[p] += 1
                    if lnstage[p] == 3:
                        del lnstage[p]
                if t is not None:
                    toks.append(ln_a(t))
                    lnstage[t] = 0
                if tok and lntok:
                    for tk in toks:
                        extra.append((len(hist) + lntok, jnp.broadcast_to(
                            tk if tk.shape[1] == 1 else jnp.concatenate([tk] * (G // 128), axis=1), (8, G))))

            def qproj(c):
                q = jnp.dot(_upk(xn_ref[hrow(c), :]), _upk(wqw_ref[...]), preferred_element_type=f32)
                qs[c] = (q * (DH ** -0.5 * LOG2E)).astype(bf16)

            def qk(c, j):
                kk = _upk(kw_ref[j * KC // 2:(j + 1) * KC // 2, :])
                st = lax.dot_general(kk, qs[c], NT, preferred_element_type=f32)
                off = pl.multiple_of(zero + j * KC, KC)
                s_refs[c % nbuf][pl.ds(off, KC), :] = st
                mm = jnp.max(st.reshape(KC // 8, 8, G), axis=0)
                maccs[c] = mm if j == 0 else jnp.maximum(maccs[c], mm)
                lastm[0] = maccs[c]

            def kcopy(hh, j):
                kw_ref[j * KC // 2:(j + 1) * KC // 2, :] = _pk(kbuf[slot(hh), j * KC:(j + 1) * KC, :])

            def vtr(hh, j):
                vt_ref[:, j * KC:(j + 1) * KC] = _pk(vbuf[slot(hh), j * KC:(j + 1) * KC, :].T)

            def pv(c, j):
                if j == 0:
                    ms[c] = jnp.broadcast_to(jnp.max(maccs[c], axis=0, keepdims=True), (8, G))
                m = ms[c]
                if lag and len(hist) >= lag:
                    for tok in hist[len(hist) - lag]:
                        m = _gate(m, tok)
                for e in [e for e in extra if e[0] <= len(hist)]:
                    m = _gate(m, e[1])
                extra[:] = [e for e in extra if e[0] > len(hist)]
                p = jnp.exp2(s_refs[c % nbuf][j * KC:(j + 1) * KC, :].reshape(KC // 8, 8, G) - m[None])
                ll = jnp.sum(p, axis=0)
                laccs[c] = ll if j == 0 else laccs[c] + ll
                oo = jnp.dot(_upk(vt_ref[:, j * KC:(j + 1) * KC]), p.reshape(KC, G).astype(bf16),
                             preferred_element_type=f32)
                oaccs[c] = oo if j == 0 else oaccs[c] + oo
                toks = []
                if 'm' in gates and lastm[0] is not None:
                    toks.append(lastm[0])
                if 'l' in gates:
                    toks.append(laccs[c])
                if 'o' in gates:
                    toks.append(oaccs[c][DH - 8:, :])
                hist.append(toks)

            def oproj(c, after=None, nsub=1):
                l = jnp.sum(laccs[c], axis=0, keepdims=True)
                o = (oaccs[c] * (1.0 / l)).T.astype(bf16)
                n = G // nsub
                for i in range(nsub):
                    rows = pl.ds((c % ng) * G + i * n, n)
                    y = jnp.dot(o[i * n:(i + 1) * n], _upk(wow_ref[...]), preferred_element_type=f32)
                    if pre:
                        acc_ref[rows, :] = y
                    else:
                        acc_ref[rows, :] += y
                    if after is not None:
                        after(i)

            def mod():
                r = _rb(r_ref[...])
                r = jnp.where(r != r, -jnp.inf, r)
                i0 = lax.broadcasted_iota(jnp.int32, r.shape, 0)
                ids = ((i0 >> 3) * 128 + lax.broadcasted_iota(jnp.int32, r.shape, 1)) * 8 + (i0 & 7)
                taken = jnp.zeros(r.shape, jnp.bool_)
                rid = lax.broadcasted_iota(jnp.int32, (C, 1), 0)
                rsel = jnp.zeros((C, 1), f32)
                idxs, rows, words = [], [], []
                for j in range(C):
                    cand = jnp.where(taken, -jnp.inf, r)
                    mx = jnp.max(cand, keepdims=True)
                    hit = jnp.logical_and(cand == mx, jnp.logical_not(taken))
                    amv = jnp.min(jnp.where(hit, ids, S - 1), keepdims=True)
                    taken = jnp.logical_or(taken, ids == amv)
                    rsel = jnp.where(rid == j, mx, rsel)
                    am = amv[0, 0]
                    idxs.append(am)
                    w = z_ref[pl.ds(lax.shift_right_logical(am, 1), 1), :]
                    words.append(w)
                    sh = ((am & 1) * 16).astype(u32)
                    rows.append(lax.shift_left(lax.shift_right_logical(w, sh), u32(16)))
                xs = pltpu.bitcast(jnp.concatenate(rows, axis=0), f32)
                xsb = xs.astype(bf16)
                a = lax.dot_general(xsb, wg_ref[...], NT, preferred_element_type=f32)
                u = lax.dot_general(xsb, wu_ref[...], NT, preferred_element_type=f32)
                hh = (a * _sigmoid(a) * u).astype(bf16)
                y = jnp.dot(hh, wd_ref[...], preferred_element_type=f32)
                zz = xs + y * _sigmoid(rsel)
                zb = lax.shift_right_logical(pltpu.bitcast(_rb(zz), u32), u32(16))
                for j in range(C):
                    row = pl.ds(lax.shift_right_logical(idxs[j], 1), 1)
                    sh = ((idxs[j] & 1) * 16).astype(u32)
                    keep = lax.shift_left(u32(0xFFFF), u32(16) - sh)
                    z_ref[row, :] = (z_ref[row, :] & keep) | lax.shift_left(zb[j:j + 1, :], sh)

            def fin(c, i, nsub, own_dma=False):
                n = G // nsub
                r0 = c * G + i * n
                for r in range(r0, r0 + n, rb):
                    hz = _upk(z_ref[r // 2:(r + rb) // 2, :]).astype(f32) * 0.5
                    g = hz * jnp.tanh(hz) + hz
                    ob_refs[c][r - c * G:r - c * G + rb, :] = (
                        x_ref[r:r + rb, :].astype(f32) + acc_ref[r:r + rb, :] * g).astype(bf16)
                if own_dma:
                    o_cp(c, i, nsub).start()
                elif i == nsub - 1:
                    o_cp(c).start()
                    ob_refs[c][pl.ds(pl.multiple_of(zero + G, 16), 16), 0:128] = jnp.zeros((16, 128), bf16)
                    if fintok:
                        done_token(ob_refs[c], fintok)

            lnq, zq = [], []
            lndone = set()
            if pre:
                x_cp(0).start()
                wq_cp(0).start()
                k_cp(0).start()
                x_cp(1).start()
                z_ref[S // 2:, 0:128] = jnp.zeros((8, 128), u32)
                for ob in ob_refs:
                    ob[G:, 0:128] = jnp.zeros((16, 128), bf16)
                for c in range(ng):
                    if p_op(c) >= B:
                        acc_ref[grow(c), :] = jnp.zeros((G, D), f32)
                x_cp(0).wait()
                v_cp(0).start()
                x_cp(2).start()
                for t in range(lnsub):
                    tick(t, False)
                while lnstage:
                    tick(None, False)
                wq_cp(0).wait()
                wo_cp(0).start()
                x_cp(3).start()
                wqw_ref[...] = _pk(wqbuf[0])
                qproj(0)
                k_cp(0).wait()
                x_cp(1).wait()
                for j in range(nk):
                    kcopy(0, j)
                for t in range(lnsub, 2 * lnsub):
                    tick(t, False)
                while lnstage:
                    tick(None, False)
                lnq = list(range(2 * lnsub, ng * lnsub))
                lo, hi = -ahead, B
            elif post:
                for i in range(3):
                    f_cp(i).wait()
                lo, hi = B, W
            else:
                for cp in (k_cp, v_cp, wq_cp, wo_cp):
                    cp(h + 1).wait()

                @pl.when(h + 3 < H)
                def _():
                    for cp in (k_cp, v_cp, wq_cp, wo_cp):
                        cp(h + 3).start()
                lo, hi = B, B + W

            if not pre:
                for i, c in enumerate(live_q):
                    qs[c] = _upk(q_c[i])
                for i, c in enumerate(live_mx):
                    maccs[c] = m_c[i]
                for i, c in enumerate(live_m):
                    ms[c] = m_c[len(live_mx) + i]
                for i, c in enumerate(live_o):
                    laccs[c] = l_c[i]
                    oaccs[c] = o_c[i]

            finq = [(c, i) for c in range(ng) if p_op(c) < B for i in range(finsub)] if post else []
            op = lambda c: max(p_op(c), w6)
            qp = lambda c: p_qproj(c) if c < 3 else min(max(p_qproj(c), w6), p_qk(c, 0) - 1)
            for pos in range(lo, hi):
                c, j = pos // nk, pos % nk
                qc, qj = (pos + ahead) // nk, (pos + ahead) % nk
                if pre and pos == w5:
                    v_cp(0).wait()
                    x_cp(2).wait()
                    for jj in range(nk):
                        vtr(0, jj)
                if pre and pos == w6:
                    for cp in (k_cp, v_cp, wq_cp, wo_cp):
                        cp(1).start()
                    wo_cp(0).wait()
                    x_cp(3).wait()
                    for cp in (k_cp, v_cp, wq_cp, wo_cp):
                        cp(2).start()
                    for i in range(3):
                        f_cp(i).start()
                    wow_ref[...] = _pk(wobuf[0])
                if not (post and qc >= ng):
                    qk(qc, qj)
                    if qc == ng - 1 and not post:
                        kcopy(h + 1, qj)
                if pos >= 0:
                    pv(c, j)
                if c == ng - 1 and not post:
                    vtr(h + 1, j)
                if pre and pos >= w5:
                    avail = [t for t in lnq if t < 3 * lnsub or pos >= w6]
                    cnt = 1
                    for n_, t in enumerate(avail):
                        dl = max(min(qp(t // lnsub), B - 1) - pos + 1, 1)
                        cnt = max(cnt, -(-(n_ + 4) // dl))
                    for p, sg in lnstage.items():
                        dl = max(min(qp(p // lnsub), B - 1) - pos + 1, 1)
                        cnt = max(cnt, -(-(3 - sg) // dl))
                    for _ in range(cnt):
                        if avail or lnstage:
                            t = avail.pop(0) if avail else None
                            if t is not None:
                                lnq.remove(t)
                            tick(t)
                    if zq and pos >= 0:
                        acc_ref[grow(zq.pop(0)), :] = jnp.zeros((G, D), f32)
                if post and pos == B + modpos:
                    mod()
                for cc in range(ng):
                    if pre and p_op(cc) < pos == op(cc):
                        oproj(cc)
                if j == opos and c - 1 >= 0 and not (pre and op(c - 1) != pos):
                    oproj(c - 1)
                    if c - 1 == ng - 1:
                        wow_ref[...] = _pk(wobuf[slot(h + 1)])
                    if post:
                        finq.extend((c - 1, i) for i in range(finsub))
                if pre:
                    for cc in range(1, ng):
                        if qp(cc) == pos:
                            assert cc in lndone, (cc, pos)
                            qproj(cc)
                elif j == qpos and not (post and c + 2 >= ng):
                    if c + 2 == ng:
                        wqw_ref[...] = _pk(wqbuf[slot(h + 1)])
                    qproj(c + 2)
                if post and pos >= B + finlag:
                    for _ in range(-(-len(finq) // (W - pos))):
                        fin(*finq.pop(0), finsub)

            if post:
                for ci in finq:
                    fin(*ci, finsub)
                oproj(ng - 1, lambda i: fin(ng - 1, i, lastsub, True), lastsub)
                for c in range(ng - 1):
                    o_cp(c).wait()
                for i in range(lastsub):
                    o_cp(ng - 1, i, lastsub).wait()
                return
            if pre:
                assert not lnq and not zq and not lnstage
                r_ref[...] = jnp.concatenate(racc, axis=0)
            sh = 0 if pre else ng
            for i, c in enumerate(live_q):
                q_c[i] = _pk(qs[c + sh])
            for i, c in enumerate(live_mx):
                m_c[i] = maccs[c + sh]
            for i, c in enumerate(live_m):
                m_c[len(live_mx) + i] = ms[c + sh]
            for i, c in enumerate(live_o):
                l_c[i] = laccs[c + sh]
                o_c[i] = oaccs[c + sh]

        zero = zero_ref[0]
        if 'P' in parts:
            segment(0, 'pre', zero)

        def mid(h, carry):
            segment(h, 'mid', jnp.minimum(h, 0))
            return carry

        if 'M' in parts:
            lax.fori_loop(0, H - 1, mid, 0)
        if 'Q' in parts:
            segment(H - 1, 'post', zero)

    def kernel_w(zero_ref, *refs):
        return kernel(*refs[:10], zero_ref, *refs[10:])

    @jax.jit
    def fn(A_x, A_k_cache, A_v_cache, A_wq, A_wo, B_x, B_w_r, B_w_gate, B_w_up, B_w_down):
        x = A_x.reshape(S, D)
        k = A_k_cache.reshape(HH, S, DH)
        v = A_v_cache.reshape(HH, S, DH)
        wr = B_w_r.reshape(1, D)
        hbm = pl.BlockSpec(memory_space=pl.ANY)
        V = pltpu.VMEM
        dma = pltpu.SemaphoreType.DMA
        out = pl.pallas_call(
            kernel_w,
            in_specs=[pl.BlockSpec(memory_space=pltpu.SMEM),
                      hbm, hbm, hbm, hbm, hbm, pl.BlockSpec(memory_space=pltpu.VMEM), hbm, hbm, hbm],
            out_specs=hbm,
            out_shape=jax.ShapeDtypeStruct((S, D), bf16),
            scratch_shapes=[
                V((S + 16, D), bf16), V((3, S, DH), bf16), V((3, S, DH), bf16), V((3, D, DH), bf16), V((3, DH, D), bf16),
                V((F, D), bf16), V((F, D), bf16), V((F, D), bf16),
                V((S // 2, D), u32), V((S // 2 + 8, D), u32), V((S + 8, D), f32), V((S // 128, 128), f32),
                V((S // 2, DH), u32), V((DH // 2, S), u32), V((D // 2, DH), u32), V((DH // 2, D), u32),
                V((len(live_mx) + len(live_m), 8, G), f32), V((len(live_o), 8, G), f32),
                V((len(live_o), DH, G), f32), V((len(live_q), G // 2, DH), u32),
                dma((nx,)), dma((3,)), dma((3,)), dma((3,)), dma((3,)), dma((3,)), dma((ng - 1 + lastsub,)),
            ] + [V((S, G), f32)] * nbuf + [V((G + 16, D), bf16)] * ng,
            compiler_params=pltpu.CompilerParams(vmem_limit_bytes=100 * 1024 * 1024),
        )(jnp.zeros((1,), jnp.int32), x, k, v, A_wq, A_wo, wr, B_w_gate.T, B_w_up.T, B_w_down)
        return out.reshape(1, S, D)

    return fn


_impl = make(**{'B':17,'lntok':0,'w6':4})


@jax.jit
def pallas_recurrent_scan__mha_block_cached__moe_arch_mod__prompt_kernel(A_x, A_k_cache, A_v_cache, A_wq, A_wo, B_x, B_w_r, B_w_gate, B_w_up, B_w_down):
    return _impl(A_x, A_k_cache, A_v_cache, A_wq, A_wo, B_x, B_w_r, B_w_gate, B_w_up, B_w_down)
```

```python
import jax
import jax.numpy as jnp
from jax import lax
import jax.experimental.pallas as pl
import jax.experimental.pallas.tpu as pltpu

S, D, HH, DH, F, C = 2048, 640, 32, 128, 1728, 8
LOG2E = 1.4426950408889634
NT = (((1,), (1,)), ((), ()))
f32 = jnp.float32
bf16 = jnp.bfloat16
u32 = jnp.uint32


def _rb(a):
    return a.astype(bf16).astype(f32)


def _gate(m, tok):
    return jnp.maximum(m, jnp.minimum(m, tok))


def _sigmoid(x):
    return 0.5 * jnp.tanh(0.5 * x) + 0.5


def _recip(d):
    r = pl.reciprocal(d, approx=True)
    r = r + r * (1.0 - d * r)
    return r + r * (1.0 - d * r)


def _pk(a):
    return pltpu.bitcast(a, u32)


def _upk(a):
    return pltpu.bitcast(a, bf16)


def make(G=256, KC=512, skew=1, lag=2, qpos=1.75, ppos=2.6, opos=14.5, nbuf=4, H=32, gates='lo', B=17.0,
         lnsub=4, modpos=3, dnpos=4, parts='PMQ', lntok=0, w5=-1, w6=4, lastsub=4, fp=0.25,
         fintok=2, gpos=(20.3, 24.3, 28.3, 32.3), lnchain=False, nob=8, reload=False, nz0=5, pinlag=1, oplag=1):
    ng = S // G
    nk = S // KC
    W = ng * nk
    ahead = nk + skew
    xsplit = (1, 1, 1, ng - 3)
    nx = len(xsplit)
    xoff = [sum(xsplit[:i]) for i in range(nx)]
    LR = G // lnsub
    GR = S // HH

    p_qproj = lambda c: (c - 2) * nk + qpos
    p_qk = lambda c, j: c * nk + j - ahead
    p_pv = lambda c, j: c * nk + j + fp
    p_pr = lambda c: (c + 1) * nk + ppos
    p_op = lambda c: (c + 1) * nk + opos
    rng = range(-2, 2 * ng + 2)
    live_q = [c for c in rng if p_qproj(c) < B <= p_qk(c, nk - 1)]
    live_mx = [c for c in rng if p_qk(c, 0) < B <= p_pv(c, 0)]
    live_m = [c for c in rng if p_pv(c, 0) < B <= p_pv(c, nk - 1)]
    live_o = [c for c in rng if p_pv(c, 0) < B <= p_pr(c)]

    def kernel(x_hbm, k_hbm, v_hbm, wq_hbm, wo_hbm, wr_hbm, wg_hbm, wu_hbm, wd_hbm, o_hbm,
               zero_ref, wr_ref, x_ref, kbuf, vbuf, wqbuf, wobuf, wg_ref, wu_ref, wd_ref,
               xn_ref, g_ref, r_ref, kw_ref, vt_ref, wqw_ref, wow_ref,
               m_c, l_c, o_c, q_c,
               xsem, hsem, fsem, osem, *rest):
        s_refs, rest = rest[:nbuf], rest[nbuf:]
        o_refs, ob_refs, acc_refs = rest[:nob], rest[nob:nob + ng], rest[nob + ng:]

        def x_cp(i):
            rows = pl.ds(xoff[i] * G, xsplit[i] * G)
            return pltpu.make_async_copy(x_hbm.at[rows, :], x_ref.at[rows, :], xsem.at[i])

        def k_cp(h):
            return pltpu.make_async_copy(k_hbm.at[h], kbuf.at[0:S, :], hsem.at[0])

        def v_cp(h):
            return pltpu.make_async_copy(v_hbm.at[h], vbuf.at[0:S, :], hsem.at[1])

        def wq_cp(h):
            col = h * DH if isinstance(h, int) else pl.multiple_of(h * DH, DH)
            return pltpu.make_async_copy(wq_hbm.at[:, pl.ds(col, DH)], wqbuf.at[0:D, :], hsem.at[2])

        def wo_cp(h):
            row = h * DH if isinstance(h, int) else pl.multiple_of(h * DH, DH)
            return pltpu.make_async_copy(wo_hbm.at[pl.ds(row, DH), :], wobuf.at[0:DH, :], hsem.at[3])

        def f_cp(i):
            src = (wg_hbm, wu_hbm, wd_hbm, wr_hbm)[i]
            dst = (wg_ref, wu_ref, wd_ref, wr_ref)[i]
            return pltpu.make_async_copy(src, dst, fsem.at[i])

        def o_cp(c, i=0, nsub=1):
            n = G // nsub
            return pltpu.make_async_copy(ob_refs[c].at[i * n:(i + 1) * n, :], o_hbm.at[pl.ds(c * G + i * n, n), :],
                                         osem.at[c + i])

        def grow(c):
            return pl.ds((c % ng) * G, G)

        def hrow(c):
            return pl.ds((c % ng) * (G // 2), G // 2)

        def segment(h, mode, zero):
            pre, post = mode == 'pre', mode == 'post'
            qs, maccs, ms, laccs, oaccs = {}, {}, {}, {}, {}
            hist = []
            lastm = [None]
            extra = []

            def after(tok):
                if tok is None:
                    return 0
                return pltpu.bitcast(tok, jnp.int32)[0, 0] & zero

            def pin(ref, lagn, val=None):
                spare = pl.ds(pl.multiple_of(zero + (ref.shape[0] - 16), 16), 16)
                ref[spare, 0:128] = jnp.zeros((16, 128), bf16) if val is None else val
                t = pltpu.bitcast(ref[spare, 0:128], f32)
                extra.append((len(hist) + lagn, jnp.concatenate([t] * (G // 128), axis=1)))

            def refill(cp, ref):
                @pl.when(h + 2 < H)
                def _():
                    cp(h + 2).start()
                pin(ref, pinlag)

            lane = lax.broadcasted_iota(jnp.int32, (8, 128), 1)
            racc = [jnp.zeros((8, 128), f32) for _ in range(S // 1024)]

            lnst = {}

            lnprev = [None]

            def ldx(t, off):
                xs = []
                for r in range(t * LR, (t + 1) * LR, 16):
                    rows = pl.ds(r, 16) if isinstance(off, int) else pl.ds(pl.multiple_of(off + r, 16), 16)
                    x16 = x_ref[rows, :].astype(f32)
                    xs += [x16[:8], x16[8:]]
                return xs

            def ln_a(t):
                xs = ldx(t, after(lnprev[0]))
                means = [jnp.sum(x, axis=-1, keepdims=True) * (1.0 / D) for x in xs]
                lnst[t] = dict(xs=xs, means=means)
                if lnchain and t >= 2 * lnsub:
                    lnprev[0] = jnp.broadcast_to(means[-1], (8, 128))
                return means[-1]

            def ln_b(t):
                st = lnst[t]
                if reload and t >= 2 * lnsub:
                    st['xs'] = ldx(t, after(jnp.broadcast_to(st['means'][0], (8, 128))) if reload == 2 else zero)
                ssq = jnp.zeros((8, 128), f32)
                for k, (x, mean) in enumerate(zip(st['xs'], st['means'])):
                    xc = x - mean
                    ssq = jnp.where(lane == k, jnp.sum(xc * xc, axis=-1, keepdims=True), ssq)
                st['inv'] = 1.0 / _rb(jnp.sqrt(_rb(_rb(ssq * (1.0 / D)) + _rb(f32(1e-5)))))
                return st['inv']

            def ln_b2(t):
                st = lnst[t]
                st['invs'] = [jnp.sum(jnp.where(lane == k, st['inv'], 0.0), axis=-1, keepdims=True)
                              for k in range(LR // 8)]
                return st['invs'][-1]

            def ln_c(t):
                st = lnst[t]
                if reload and t >= 2 * lnsub:
                    st['xs'] = ldx(t, after(st['inv']) if reload == 2 else zero + zero)
                wr = jnp.broadcast_to(wr_ref[...].astype(f32).reshape(1, D), (8, D))
                for k in range(0, LR // 8, 2):
                    xn = jnp.concatenate([_rb(st['xs'][kk] - _rb(st['means'][kk])) * st['invs'][kk]
                                          for kk in (k, k + 1)], axis=0)
                    xnb = xn.astype(bf16)
                    r = t * LR + k * 8
                    xn_ref[r // 2:r // 2 + 8, :] = _pk(xnb)
                    xr = xnb.astype(f32)
                    for kk in (0, 1):
                        rg = r // 8 + kk
                        rr = jnp.sum(xr[kk * 8:kk * 8 + 8] * wr, axis=-1, keepdims=True)
                        racc[rg // 128] = jnp.where(lane == rg % 128, rr, racc[rg // 128])
                del lnst[t]
                if (t + 1) % lnsub == 0:
                    lndone.add(t // lnsub)
                return racc[(t * LR) // 1024]

            lnstage = {}

            def tick(t, tok=True):
                toks = []
                for p in sorted(lnstage):
                    toks.append((ln_b, ln_b2, ln_c)[lnstage[p]](p))
                    lnstage[p] += 1
                    if lnstage[p] == 3:
                        del lnstage[p]
                if t is not None:
                    toks.append(ln_a(t))
                    lnstage[t] = 0
                if tok and lntok:
                    for tk in toks:
                        extra.append((len(hist) + lntok, jnp.broadcast_to(
                            tk if tk.shape[1] == 1 else jnp.concatenate([tk] * (G // 128), axis=1), (8, G))))

            def qproj(c):
                q = jnp.dot(_upk(xn_ref[hrow(c), :]), _upk(wqw_ref[...]), preferred_element_type=f32)
                qs[c] = (q * (DH ** -0.5 * LOG2E)).astype(bf16)

            def qk(c, j):
                kk = _upk(kw_ref[j * KC // 2:(j + 1) * KC // 2, :])
                st = lax.dot_general(kk, qs[c], NT, preferred_element_type=f32)
                off = pl.multiple_of(zero + j * KC, KC)
                s_refs[c % nbuf][pl.ds(off, KC), :] = st
                mm = jnp.max(st.reshape(KC // 8, 8, G), axis=0)
                maccs[c] = mm if j == 0 else jnp.maximum(maccs[c], mm)
                lastm[0] = maccs[c]

            def kcopy(hh, j):
                kw_ref[j * KC // 2:(j + 1) * KC // 2, :] = _pk(kbuf[j * KC:(j + 1) * KC, :])

            def vtr(hh, j):
                vt_ref[:, j * KC:(j + 1) * KC] = _pk(vbuf[j * KC:(j + 1) * KC, :].T)

            def pv(c, j):
                if j == 0:
                    ms[c] = jnp.broadcast_to(jnp.max(maccs[c], axis=0, keepdims=True), (8, G))
                m = ms[c]
                if lag and len(hist) >= lag:
                    for tok in hist[len(hist) - lag]:
                        m = _gate(m, tok)
                for e in [e for e in extra if e[0] <= len(hist)]:
                    m = _gate(m, e[1])
                extra[:] = [e for e in extra if e[0] > len(hist)]
                p = jnp.exp2(s_refs[c % nbuf][j * KC:(j + 1) * KC, :].reshape(KC // 8, 8, G) - m[None])
                ll = jnp.sum(p, axis=0)
                laccs[c] = ll if j == 0 else laccs[c] + ll
                oo = jnp.dot(_upk(vt_ref[:, j * KC:(j + 1) * KC]), p.reshape(KC, G).astype(bf16),
                             preferred_element_type=f32)
                oaccs[c] = oo if j == 0 else oaccs[c] + oo
                toks = []
                if 'm' in gates and lastm[0] is not None:
                    toks.append(lastm[0])
                if 'l' in gates:
                    toks.append(laccs[c])
                if 'o' in gates:
                    toks.append(oaccs[c][DH - 8:, :])
                hist.append(toks)

            def oprep(c):
                l = jnp.sum(laccs[c], axis=0, keepdims=True)
                o_refs[c % nob][...] = _pk((oaccs[c] * (1.0 / l)).T.astype(bf16))

            def oproj(c, nsub=1):
                n = G // nsub
                for i in range(nsub):
                    rows = pl.ds(i * n, n)
                    y = jnp.dot(_upk(o_refs[c % nob][i * n // 2:(i + 1) * n // 2, :]), _upk(wow_ref[...]),
                                preferred_element_type=f32)
                    if pre:
                        acc_refs[c][rows, :] = y
                    elif not post:
                        acc_refs[c % ng][rows, :] += y
                    else:
                        for r in range(i * n, (i + 1) * n, 16):
                            g = _upk(g_ref[(c * G + r) // 2:(c * G + r) // 2 + 8, :]).astype(f32)
                            sv = acc_refs[c][r:r + 16, :] + y[r - i * n:r - i * n + 16]
                            o = (x_ref[c * G + r:c * G + r + 16, :].astype(f32) + sv * g).astype(bf16)
                            ob_refs[c][r:r + 16, :] = o
                        o_cp(c, i, nsub).start()
                if post and nsub == 1 and fintok:
                    pin(ob_refs[c], fintok, o[:, D - 128:])

            md = {}

            def mod():
                r = _rb(r_ref[...]) + 0.0
                i0 = lax.broadcasted_iota(jnp.int32, r.shape, 0)
                ids = ((i0 >> 3) * 128 + lax.broadcasted_iota(jnp.int32, r.shape, 1)) * 8 + (i0 & 7)
                bits = pltpu.bitcast(r, jnp.int32)
                hi = jnp.where(bits < 0, bits ^ 0x7FFF0000, bits)
                hi = jnp.where(r != r, jnp.int32(-2 ** 31), hi)
                key = hi | (S - ids)
                rid = lax.broadcasted_iota(jnp.int32, (C, 1), 0)
                ksel = jnp.zeros((C, 1), jnp.int32)
                idxs, rows = [], []
                for j in range(C):
                    mx = jnp.max(key, keepdims=True)
                    key = jnp.where(key == mx, jnp.int32(-2 ** 31), key)
                    ksel = jnp.where(rid == j, mx, ksel)
                    am = S - (mx[0, 0] & 0xFFFF)
                    idxs.append(am)
                    w = xn_ref[pl.ds(lax.shift_right_logical(am, 1), 1), :]
                    sh = ((am & 1) * 16).astype(u32)
                    rows.append(lax.shift_left(lax.shift_right_logical(w, sh), u32(16)))
                xs = pltpu.bitcast(jnp.concatenate(rows, axis=0), f32)
                xsb = xs.astype(bf16)
                ksel = ksel & jnp.int32(-65536)
                rsel = pltpu.bitcast(jnp.broadcast_to(jnp.where(ksel < 0, ksel ^ 0x7FFF0000, ksel), (C, 128)), f32)[:, 0:1]
                md.update(xs=xs, xsb=xsb, idxs=idxs, rsel=rsel)

            def mod_gu():
                xsb = md['xsb']
                a = lax.dot_general(xsb, wg_ref[...], NT, preferred_element_type=f32)
                u = lax.dot_general(xsb, wu_ref[...], NT, preferred_element_type=f32)
                md['hh'] = (a * _sigmoid(a) * u).astype(bf16)

            def mod_dn():
                xs, idxs, rsel = md['xs'], md['idxs'], md['rsel']
                y = jnp.dot(md['hh'], wd_ref[...], preferred_element_type=f32)
                zz = xs + y * _sigmoid(rsel)
                hz = _rb(zz) * 0.5
                zb = lax.shift_right_logical(pltpu.bitcast(_rb(hz * jnp.tanh(hz) + hz), u32), u32(16))
                for j in range(C):
                    row = pl.ds(lax.shift_right_logical(idxs[j], 1), 1)
                    sh = ((idxs[j] & 1) * 16).astype(u32)
                    keep = lax.shift_left(u32(0xFFFF), u32(16) - sh)
                    g_ref[row, :] = (g_ref[row, :] & keep) | lax.shift_left(zb[j:j + 1, :], sh)

            def gate_silu(k):
                if pre:
                    rows = pl.ds((H - 1) * (GR // 2) + k * 8, 8)
                else:
                    rows = pl.ds(pl.multiple_of(h * (GR // 2) + k * 8 + after(hist[-1][-1][:, :128]), 8), 8)
                hz = _upk(xn_ref[rows, :]).astype(f32) * 0.5
                g_ref[rows, :] = _pk((hz * jnp.tanh(hz) + hz).astype(bf16))

            lnq = []
            lndone = set()
            if pre:
                x_cp(0).start()
                f_cp(3).start()
                wq_cp(0).start()
                k_cp(0).start()
                x_cp(1).start()
                zq = [c for c in range(ng) if p_op(c) >= B]
                for c in zq[:nz0]:
                    acc_refs[c][...] = jnp.zeros((G, D), f32)
                x_cp(0).wait()
                f_cp(3).wait()
                v_cp(0).start()
                x_cp(2).start()
                for t in range(lnsub):
                    tick(t, False)
                while lnstage:
                    tick(None, False)
                wq_cp(0).wait()
                wo_cp(0).start()
                x_cp(3).start()
                wqw_ref[...] = _pk(wqbuf[0:D, :])
                qproj(0)
                for c in zq[nz0:]:
                    acc_refs[c][...] = jnp.zeros((G, D), f32)
                k_cp(0).wait()
                x_cp(1).wait()
                for j in range(nk):
                    kcopy(0, j)
                for t in range(lnsub, 2 * lnsub):
                    tick(t, False)
                while lnstage:
                    tick(None, False)
                lnq = list(range(2 * lnsub, ng * lnsub))
                lo, hi = -ahead, B
            elif post:
                for i in range(3):
                    f_cp(i).wait()
                lo, hi = B, W
            else:
                for cp in (k_cp, v_cp, wq_cp, wo_cp):
                    cp(h + 1).wait()
                lo, hi = B, B + W

            if not pre:
                for i, c in enumerate(live_q):
                    qs[c] = _upk(q_c[i])
                for i, c in enumerate(live_mx):
                    maccs[c] = m_c[i]
                for i, c in enumerate(live_m):
                    ms[c] = m_c[len(live_mx) + i]
                for i, c in enumerate(live_o):
                    laccs[c] = l_c[i]
                    oaccs[c] = o_c[i]

            assert p_op(0) >= B or not post
            pr = lambda c: max(B, (c + 1) * nk + 0.3) if post and p_pr(c) >= B else p_pr(c)
            if post:
                op = lambda c: max(pr(c) + oplag, int(B) + dnpos + 1.5 + c)
            else:
                op = lambda c: max(p_op(c), w6 + 0.5) if pre else p_op(c)
            qp = lambda c: min(max(p_qproj(c), w6 + 0.75), p_qk(c, 0) - 0.25) if pre and c >= 3 else p_qproj(c)

            def ev_qk(c, j):
                qk(c, j)
                if c == ng - 1 and not post:
                    kcopy(h + 1, j)
                    if j == nk - 1:
                        refill(k_cp, kbuf)

            def ev_pv(c, j):
                pv(c, j)
                if c == ng - 1 and not post:
                    vtr(h + 1, j)
                    if j == nk - 1:
                        refill(v_cp, vbuf)

            def ev_op(c):
                oproj(c)
                if c == ng - 1:
                    wow_ref[...] = _pk(wobuf[0:DH, :])
                    refill(wo_cp, wobuf)

            def ev_qp(c):
                if c == ng:
                    wqw_ref[...] = _pk(wqbuf[0:D, :])
                    refill(wq_cp, wqbuf)
                assert not pre or c in lndone, c
                qproj(c)

            def ev_w5():
                v_cp(0).wait()
                x_cp(2).wait()
                for jj in range(nk):
                    vtr(0, jj)

            def ev_w6():
                for cp in (k_cp, v_cp, wq_cp):
                    cp(1).start()
                wo_cp(0).wait()
                x_cp(3).wait()
                wow_ref[...] = _pk(wobuf[0:DH, :])
                wo_cp(1).start()
                pin(wobuf, 2)
                for i in range(3):
                    f_cp(i).start()

            def ev_ln(pos):
                avail = [t for t in lnq if t < 3 * lnsub or pos >= w6]
                left = lambda c: max(len([1 for tt in lntimes if pos <= tt < min(qp(c), B)]), 1)
                cnt = 1
                for n_, t in enumerate(avail):
                    cnt = max(cnt, -(-(n_ + 4) // left(t // lnsub)))
                for p, sg in lnstage.items():
                    cnt = max(cnt, -(-(3 - sg) // left(p // lnsub)))
                for _ in range(cnt):
                    if avail or lnstage:
                        t = avail.pop(0) if avail else None
                        if t is not None:
                            lnq.remove(t)
                        tick(t)

            cmax = ng - 1 if post or pre else 2 * ng + 1
            ev = []
            for c in range(0, cmax + 1):
                for j in range(nk):
                    ev.append((p_qk(c, j), ev_qk, (c, j)))
                    ev.append((p_pv(c, j), ev_pv, (c, j)))
                if not (post and c == ng - 1):
                    ev.append((op(c), ev_op, (c,)))
                    ev.append((pr(c), oprep, (c,)))
                if c >= 1:
                    ev.append((qp(c), ev_qp, (c,)))
            if pre:
                lntimes = [t + 0.4 for t in range(w5, W)]
                ev += [(w5 - 0.01, ev_w5, ()), (w6 - 0.01, ev_w6, ())]
                ev += [(t, ev_ln, (t,)) for t in lntimes]
            if not post:
                ev += [(B - 0.001 if pre else gpos[k], gate_silu, (k,)) for k in range(GR // 16)]
            if post:
                ev += [(B, mod, ()), (int(B) + modpos + 0.4, mod_gu, ()),
                       (int(B) + dnpos + 0.45, mod_dn, ())]
            for t, f, a in sorted([e for e in ev if lo <= e[0] < hi], key=lambda e: e[0]):
                f(*a)

            if post:
                oprep(ng - 1)
                oproj(ng - 1, lastsub)
                for c in range(ng - 1):
                    o_cp(c).wait()
                for i in range(lastsub):
                    o_cp(ng - 1, i, lastsub).wait()
                return
            if pre:
                assert not lnq and not lnstage
                r_ref[...] = jnp.concatenate(racc, axis=0)
            sh = 0 if pre else ng
            for i, c in enumerate(live_q):
                q_c[i] = _pk(qs[c + sh])
            for i, c in enumerate(live_mx):
                m_c[i] = maccs[c + sh]
            for i, c in enumerate(live_m):
                m_c[len(live_mx) + i] = ms[c + sh]
            for i, c in enumerate(live_o):
                l_c[i] = laccs[c + sh]
                o_c[i] = oaccs[c + sh]

        zero = zero_ref[0]
        if 'P' in parts:
            segment(0, 'pre', zero)

        def mid(h, carry):
            segment(h, 'mid', jnp.minimum(h, 0))
            return carry

        if 'M' in parts:
            lax.fori_loop(0, H - 1, mid, 0)
        if 'Q' in parts:
            segment(H - 1, 'post', zero)

    def kernel_w(zero_ref, *refs):
        return kernel(*refs[:10], zero_ref, *refs[10:])

    @jax.jit
    def fn(A_x, A_k_cache, A_v_cache, A_wq, A_wo, B_x, B_w_r, B_w_gate, B_w_up, B_w_down):
        x = A_x.reshape(S, D)
        k = A_k_cache.reshape(HH, S, DH)
        v = A_v_cache.reshape(HH, S, DH)
        wr = B_w_r
        hbm = pl.BlockSpec(memory_space=pl.ANY)
        V = pltpu.VMEM
        dma = pltpu.SemaphoreType.DMA
        out = pl.pallas_call(
            kernel_w,
            in_specs=[pl.BlockSpec(memory_space=pltpu.SMEM),
                      hbm, hbm, hbm, hbm, hbm, hbm, hbm, hbm, hbm],
            out_specs=hbm,
            out_shape=jax.ShapeDtypeStruct((S, D), bf16),
            scratch_shapes=[
                V((D,), bf16), V((S, D), bf16), V((S + 16, DH), bf16), V((S + 16, DH), bf16), V((D + 16, DH), bf16), V((DH + 16, D), bf16),
                V((F, D), bf16), V((F, D), bf16), V((F, D), bf16),
                V((S // 2, D), u32), V((S // 2, D), u32), V((S // 128, 128), f32),
                V((S // 2, DH), u32), V((DH // 2, S), u32), V((D // 2, DH), u32), V((DH // 2, D), u32),
                V((len(live_mx) + len(live_m), 8, G), f32), V((len(live_o), 8, G), f32),
                V((len(live_o), DH, G), f32), V((len(live_q), G // 2, DH), u32),
                dma((nx,)), dma((4,)), dma((4,)), dma((ng - 1 + lastsub,)),
            ] + [V((S, G), f32)] * nbuf + [V((G // 2, DH), u32)] * nob + [V((G + 16, D), bf16)] * ng + [V((G, D), f32)] * ng,
            compiler_params=pltpu.CompilerParams(vmem_limit_bytes=100 * 1024 * 1024),
        )(jnp.zeros((1,), jnp.int32), x, k, v, A_wq, A_wo, wr, B_w_gate.T, B_w_up.T, B_w_down)
        return out.reshape(1, S, D)

    return fn


_impl = make(**{})


@jax.jit
def pallas_recurrent_scan__mha_block_cached__moe_arch_mod__prompt_kernel(A_x, A_k_cache, A_v_cache, A_wq, A_wo, B_x, B_w_r, B_w_gate, B_w_up, B_w_down):
    return _impl(A_x, A_k_cache, A_v_cache, A_wq, A_wo, B_x, B_w_r, B_w_gate, B_w_up, B_w_down)
```

```python
import jax
import jax.numpy as jnp
from jax import lax
import jax.experimental.pallas as pl
import jax.experimental.pallas.tpu as pltpu

S, D, HH, DH, F, C = 2048, 640, 32, 128, 1728, 8
LOG2E = 1.4426950408889634
NT = (((1,), (1,)), ((), ()))
f32 = jnp.float32
bf16 = jnp.bfloat16
u32 = jnp.uint32


def _rb(a):
    return a.astype(bf16).astype(f32)


def _gate(m, tok):
    return jnp.maximum(m, jnp.minimum(m, tok))


def _sigmoid(x):
    return 0.5 * jnp.tanh(0.5 * x) + 0.5


def _recip(d):
    r = pl.reciprocal(d, approx=True)
    r = r + r * (1.0 - d * r)
    return r + r * (1.0 - d * r)


def _pk(a):
    return pltpu.bitcast(a, u32)


def _upk(a):
    return pltpu.bitcast(a, bf16)


def make(G=256, KC=512, skew=1, lag=2, qpos=1.75, ppos=2.6, opos=10.5, nbuf=4, H=32, gates='lo', B=13.0,
         lnsub=4, modpos=3, dnpos=4, parts='PMQ', lntok=0, w5=-1, w6=4, lastsub=4, fp=0.25,
         fintok=2, gpos=(20.3, 24.3, 28.3, 32.3), nob=8, nz0=5, pinlag=1, oplag=1, gmode='none'):
    ng = S // G
    nk = S // KC
    W = ng * nk
    ahead = nk + skew
    xsplit = (1, 1, 1, ng - 3)
    nx = len(xsplit)
    xoff = [sum(xsplit[:i]) for i in range(nx)]
    LR = G // lnsub
    GR = S // HH

    p_qproj = lambda c: (c - 2) * nk + qpos
    p_qk = lambda c, j: c * nk + j - ahead
    p_pv = lambda c, j: c * nk + j + fp
    p_pr = lambda c: (c + 1) * nk + ppos
    p_op = lambda c: (c + 1) * nk + opos
    rng = range(-2, 2 * ng + 2)
    live_q = [c for c in rng if p_qproj(c) < B <= p_qk(c, nk - 1)]
    live_mx = [c for c in rng if p_qk(c, 0) < B <= p_pv(c, 0)]
    live_m = [c for c in rng if p_pv(c, 0) < B <= p_pv(c, nk - 1)]
    live_o = [c for c in rng if p_pv(c, 0) < B <= p_pr(c)]

    def kernel(x_hbm, k_hbm, v_hbm, wq_hbm, wo_hbm, wr_hbm, wg_hbm, wu_hbm, wd_hbm, o_hbm,
               zero_ref, wr_ref, wrf_ref, x_ref, kbuf, vbuf, wqbuf, wobuf, wg_ref, wu_ref, wd_ref,
               xn_ref, g_ref, r_ref, kw_ref, vt_ref, wqw_ref, wow_ref,
               m_c, l_c, o_c, q_c,
               xsem, hsem, fsem, osem, *rest):
        s_refs, rest = rest[:nbuf], rest[nbuf:]
        o_refs, ob_refs, acc_refs = rest[:nob], rest[nob:nob + ng], rest[nob + ng:]

        def x_cp(i):
            rows = pl.ds(xoff[i] * G, xsplit[i] * G)
            return pltpu.make_async_copy(x_hbm.at[rows, :], x_ref.at[rows, :], xsem.at[i])

        def k_cp(h):
            return pltpu.make_async_copy(k_hbm.at[h], kbuf.at[0:S, :], hsem.at[0])

        def v_cp(h):
            return pltpu.make_async_copy(v_hbm.at[h], vbuf.at[0:S, :], hsem.at[1])

        def wq_cp(h):
            col = h * DH if isinstance(h, int) else pl.multiple_of(h * DH, DH)
            return pltpu.make_async_copy(wq_hbm.at[:, pl.ds(col, DH)], wqbuf.at[0:D, :], hsem.at[2])

        def wo_cp(h):
            row = h * DH if isinstance(h, int) else pl.multiple_of(h * DH, DH)
            return pltpu.make_async_copy(wo_hbm.at[pl.ds(row, DH), :], wobuf.at[0:DH, :], hsem.at[3])

        def f_cp(i):
            src = (wg_hbm, wu_hbm, wd_hbm, wr_hbm)[i]
            dst = (wg_ref, wu_ref, wd_ref, wr_ref)[i]
            return pltpu.make_async_copy(src, dst, fsem.at[i])

        def o_cp(c, i=0, nsub=1):
            n = G // nsub
            return pltpu.make_async_copy(ob_refs[c].at[i * n:(i + 1) * n, :], o_hbm.at[pl.ds(c * G + i * n, n), :],
                                         osem.at[c + i])

        def grow(c):
            return pl.ds((c % ng) * G, G)

        def hrow(c):
            return pl.ds((c % ng) * (G // 2), G // 2)

        def segment(h, mode, zero):
            pre, post = mode == 'pre', mode == 'post'
            qs, maccs, ms, laccs, oaccs = {}, {}, {}, {}, {}
            hist = []
            lastm = [None]
            extra = []

            def after(tok):
                if tok is None:
                    return 0
                return pltpu.bitcast(tok, jnp.int32)[0, 0] & zero

            def pin(ref, lagn, val=None):
                spare = pl.ds(pl.multiple_of(zero + (ref.shape[0] - 16), 16), 16)
                ref[spare, 0:128] = jnp.zeros((16, 128), bf16) if val is None else val
                t = pltpu.bitcast(ref[spare, 0:128], f32)
                extra.append((len(hist) + lagn, jnp.concatenate([t] * (G // 128), axis=1)))

            def refill(cp, ref):
                @pl.when(h + 2 < H)
                def _():
                    cp(h + 2).start()
                pin(ref, pinlag)

            lane = lax.broadcasted_iota(jnp.int32, (8, 128), 1)

            lnst = {}

            def ln_a(t):
                xs = []
                for r in range(t * LR, (t + 1) * LR, 16):
                    x16 = x_ref[r:r + 16, :].astype(f32)
                    xs += [x16[:8], x16[8:]]
                means = [jnp.sum(x, axis=-1, keepdims=True) * (1.0 / D) for x in xs]
                lnst[t] = dict(xs=xs, means=means)
                return means[-1]

            def ln_b(t):
                st = lnst[t]
                ssq = jnp.zeros((8, 128), f32)
                dm = jnp.zeros((8, 128), f32)
                ds = []
                for k, (x, mean) in enumerate(zip(st['xs'], st['means'])):
                    mk = _rb(mean)
                    d = x - mk
                    ds.append(d)
                    ssq = jnp.where(lane == k, jnp.sum(d * d, axis=-1, keepdims=True), ssq)
                    dm = jnp.where(lane == k, mean - mk, dm)
                st['d'] = [jnp.concatenate(ds[k:k + 2], axis=0).astype(bf16) for k in range(0, LR // 8, 2)]
                var = jnp.maximum(ssq * (1.0 / D) - dm * dm, 0.0)
                st['inv'] = 1.0 / _rb(jnp.sqrt(_rb(_rb(var) + _rb(f32(1e-5)))))
                return st['inv']

            def ln_b2(t):
                st = lnst[t]
                st['invs'] = [jnp.sum(jnp.where(lane == k, st['inv'], 0.0), axis=-1, keepdims=True)
                              for k in range(LR // 8)]
                return st['invs'][-1]

            def ln_c(t):
                st = lnst.pop(t)
                for k in range(0, LR // 8, 2):
                    d = st['d'][k // 2].astype(f32)
                    xn = jnp.concatenate([d[:8] * st['invs'][k], d[8:] * st['invs'][k + 1]], axis=0)
                    r = t * LR + k * 8
                    xn_ref[r // 2:r // 2 + 8, :] = _pk(xn.astype(bf16))
                if (t + 1) % lnsub == 0:
                    lndone.add(t // lnsub)
                return xn[8:, D - 128:]

            lnstage = {}

            def tick(t, tok=True):
                toks = []
                for p in sorted(lnstage):
                    toks.append((ln_b, ln_b2, ln_c)[lnstage[p]](p))
                    lnstage[p] += 1
                    if lnstage[p] == 3:
                        del lnstage[p]
                if t is not None:
                    toks.append(ln_a(t))
                    lnstage[t] = 0
                if tok and lntok:
                    for tk in toks:
                        extra.append((len(hist) + lntok, jnp.broadcast_to(
                            tk if tk.shape[1] == 1 else jnp.concatenate([tk] * (G // 128), axis=1), (8, G))))

            def qproj(c):
                q = jnp.dot(_upk(xn_ref[hrow(c), :]), _upk(wqw_ref[...]), preferred_element_type=f32)
                qs[c] = (q * (DH ** -0.5 * LOG2E)).astype(bf16)

            def qk(c, j):
                kk = _upk(kw_ref[j * KC // 2:(j + 1) * KC // 2, :])
                st = lax.dot_general(kk, qs[c], NT, preferred_element_type=f32)
                off = pl.multiple_of(zero + j * KC, KC)
                s_refs[c % nbuf][pl.ds(off, KC), :] = st
                mm = jnp.max(st.reshape(KC // 8, 8, G), axis=0)
                maccs[c] = mm if j == 0 else jnp.maximum(maccs[c], mm)
                lastm[0] = maccs[c]

            def kcopy(hh, j):
                kw_ref[j * KC // 2:(j + 1) * KC // 2, :] = _pk(kbuf[j * KC:(j + 1) * KC, :])

            def vtr(hh, j):
                vt_ref[:, j * KC:(j + 1) * KC] = _pk(vbuf[j * KC:(j + 1) * KC, :].T)

            def pv(c, j):
                if j == 0:
                    ms[c] = jnp.broadcast_to(jnp.max(maccs[c], axis=0, keepdims=True), (8, G))
                m = ms[c]
                if lag and len(hist) >= lag:
                    for tok in hist[len(hist) - lag]:
                        m = _gate(m, tok)
                for e in [e for e in extra if e[0] <= len(hist)]:
                    m = _gate(m, e[1])
                extra[:] = [e for e in extra if e[0] > len(hist)]
                p = jnp.exp2(s_refs[c % nbuf][j * KC:(j + 1) * KC, :].reshape(KC // 8, 8, G) - m[None])
                ll = jnp.sum(p, axis=0)
                laccs[c] = ll if j == 0 else laccs[c] + ll
                oo = jnp.dot(_upk(vt_ref[:, j * KC:(j + 1) * KC]), p.reshape(KC, G).astype(bf16),
                             preferred_element_type=f32)
                oaccs[c] = oo if j == 0 else oaccs[c] + oo
                toks = []
                if 'm' in gates and lastm[0] is not None:
                    toks.append(lastm[0])
                if 'l' in gates:
                    toks.append(laccs[c])
                if 'o' in gates:
                    toks.append(oaccs[c][DH - 8:, :])
                hist.append(toks)

            def oprep(c):
                l = jnp.sum(laccs[c], axis=0, keepdims=True)
                o_refs[c % nob][...] = _pk((oaccs[c] * (1.0 / l)).T.astype(bf16))

            def oproj(c, nsub=1):
                n = G // nsub
                for i in range(nsub):
                    rows = pl.ds(i * n, n)
                    y = jnp.dot(_upk(o_refs[c % nob][i * n // 2:(i + 1) * n // 2, :]), _upk(wow_ref[...]),
                                preferred_element_type=f32)
                    if pre:
                        acc_refs[c][rows, :] = y
                    elif not post:
                        acc_refs[c % ng][rows, :] += y
                    else:
                        for r in range(i * n, (i + 1) * n, 16):
                            g = _upk(g_ref[(c * G + r) // 2:(c * G + r) // 2 + 8, :]).astype(f32)
                            sv = acc_refs[c][r:r + 16, :] + y[r - i * n:r - i * n + 16]
                            o = (x_ref[c * G + r:c * G + r + 16, :].astype(f32) + sv * g).astype(bf16)
                            ob_refs[c][r:r + 16, :] = o
                        o_cp(c, i, nsub).start()
                if post and nsub == 1 and fintok:
                    pin(ob_refs[c], fintok, o[:, D - 128:])

            md = {}

            def mod():
                r = _rb(r_ref[...]) + 0.0
                i0 = lax.broadcasted_iota(jnp.int32, r.shape, 0)
                ids = ((i0 >> 3) * 128 + lax.broadcasted_iota(jnp.int32, r.shape, 1)) * 8 + (i0 & 7)
                bits = pltpu.bitcast(r, jnp.int32)
                hi = jnp.where(bits < 0, bits ^ 0x7FFF0000, bits)
                hi = jnp.where(r != r, jnp.int32(-2 ** 31), hi)
                key = hi | (S - ids)
                rid = lax.broadcasted_iota(jnp.int32, (C, 1), 0)
                ksel = jnp.zeros((C, 1), jnp.int32)
                idxs, rows = [], []
                for j in range(C):
                    mx = jnp.max(key, keepdims=True)
                    key = jnp.where(key == mx, jnp.int32(-2 ** 31), key)
                    ksel = jnp.where(rid == j, mx, ksel)
                    am = S - (mx[0, 0] & 0xFFFF)
                    idxs.append(am)
                    w = xn_ref[pl.ds(lax.shift_right_logical(am, 1), 1), :]
                    sh = ((am & 1) * 16).astype(u32)
                    rows.append(lax.shift_left(lax.shift_right_logical(w, sh), u32(16)))
                xs = pltpu.bitcast(jnp.concatenate(rows, axis=0), f32)
                xsb = xs.astype(bf16)
                ksel = ksel & jnp.int32(-65536)
                rsel = pltpu.bitcast(jnp.broadcast_to(jnp.where(ksel < 0, ksel ^ 0x7FFF0000, ksel), (C, 128)), f32)[:, 0:1]
                md.update(xs=xs, xsb=xsb, idxs=idxs, rsel=rsel)

            def mod_gu():
                xsb = md['xsb']
                a = lax.dot_general(xsb, wg_ref[...], NT, preferred_element_type=f32)
                u = lax.dot_general(xsb, wu_ref[...], NT, preferred_element_type=f32)
                md['hh'] = (a * _sigmoid(a) * u).astype(bf16)

            def mod_dn():
                xs, idxs, rsel = md['xs'], md['idxs'], md['rsel']
                y = jnp.dot(md['hh'], wd_ref[...], preferred_element_type=f32)
                zz = xs + y * _sigmoid(rsel)
                hz = _rb(zz) * 0.5
                zb = lax.shift_right_logical(pltpu.bitcast(_rb(hz * jnp.tanh(hz) + hz), u32), u32(16))
                for j in range(C):
                    row = pl.ds(lax.shift_right_logical(idxs[j], 1), 1)
                    sh = ((idxs[j] & 1) * 16).astype(u32)
                    keep = lax.shift_left(u32(0xFFFF), u32(16) - sh)
                    g_ref[row, :] = (g_ref[row, :] & keep) | lax.shift_left(zb[j:j + 1, :], sh)

            def gate_silu(k):
                if pre:
                    rg = (H - 1) * (GR // 8) + 2 * k
                    rows = pl.ds(rg * 4, 8)
                else:
                    rg = h * (GR // 8) + 2 * k
                    rows = pl.ds(pl.multiple_of(rg * 4 + (after(hist[-1][-1][:, :128]) if gmode == 'after' else 0), 8), 8)
                xp = xn_ref[rows, :]
                if gmode == 'or' and not pre:
                    zz = pltpu.bitcast(hist[-1][-1][:, :128], u32) & zero.astype(u32)
                    xp = xp | jnp.concatenate([zz] * (D // 128), axis=1)
                xn = _upk(xp).astype(f32)
                hz = xn * 0.5
                g_ref[rows, :] = _pk((hz * jnp.tanh(hz) + hz).astype(bf16))
                xw = xn * wrf_ref[...]
                rr = [jnp.sum(xw[kk * 8:kk * 8 + 8], axis=-1, keepdims=True) for kk in (0, 1)]
                for v in range(S // 1024):
                    r = r_ref[v * 8:v * 8 + 8, :]
                    for kk in (0, 1):
                        r = jnp.where(lane == rg + (kk - v * 128), rr[kk], r)
                    r_ref[v * 8:v * 8 + 8, :] = r

            lnq = []
            lndone = set()
            if pre:
                x_cp(0).start()
                f_cp(3).start()
                wq_cp(0).start()
                k_cp(0).start()
                x_cp(1).start()
                zq = [c for c in range(ng) if p_op(c) >= B]
                for c in zq[:nz0]:
                    acc_refs[c][...] = jnp.zeros((G, D), f32)
                x_cp(0).wait()
                f_cp(3).wait()
                wrf_ref[...] = jnp.broadcast_to(wr_ref[...].astype(f32).reshape(1, D), (16, D))
                r_ref[...] = jnp.zeros(r_ref.shape, f32)
                v_cp(0).start()
                x_cp(2).start()
                for t in range(lnsub):
                    tick(t, False)
                while lnstage:
                    tick(None, False)
                wq_cp(0).wait()
                wo_cp(0).start()
                x_cp(3).start()
                wqw_ref[...] = _pk(wqbuf[0:D, :])
                qproj(0)
                for c in zq[nz0:]:
                    acc_refs[c][...] = jnp.zeros((G, D), f32)
                k_cp(0).wait()
                x_cp(1).wait()
                for j in range(nk):
                    kcopy(0, j)
                for t in range(lnsub, 2 * lnsub):
                    tick(t, False)
                while lnstage:
                    tick(None, False)
                lnq = list(range(2 * lnsub, ng * lnsub))
                lo, hi = -ahead, B
            elif post:
                for i in range(3):
                    f_cp(i).wait()
                lo, hi = B, W
            else:
                for cp in (k_cp, v_cp, wq_cp, wo_cp):
                    cp(h + 1).wait()
                lo, hi = B, B + W

            if not pre:
                for i, c in enumerate(live_q):
                    qs[c] = _upk(q_c[i])
                for i, c in enumerate(live_mx):
                    maccs[c] = m_c[i]
                for i, c in enumerate(live_m):
                    ms[c] = m_c[len(live_mx) + i]
                for i, c in enumerate(live_o):
                    laccs[c] = l_c[i]
                    oaccs[c] = o_c[i]

            assert p_op(0) >= B or not post
            pr = lambda c: max(B, (c + 1) * nk + 0.3) if post and p_pr(c) >= B else p_pr(c)
            if post:
                op = lambda c: max(pr(c) + oplag, int(B) + dnpos + 1.5 + c)
            else:
                op = lambda c: max(p_op(c), w6 + 0.5) if pre else p_op(c)
            qp = lambda c: min(max(p_qproj(c), w6 + 0.75), p_qk(c, 0) - 0.25) if pre and c >= 3 else p_qproj(c)

            def ev_qk(c, j):
                qk(c, j)
                if c == ng - 1 and not post:
                    kcopy(h + 1, j)
                    if j == nk - 1:
                        refill(k_cp, kbuf)

            def ev_pv(c, j):
                pv(c, j)
                if c == ng - 1 and not post:
                    vtr(h + 1, j)
                    if j == nk - 1:
                        refill(v_cp, vbuf)

            def ev_op(c):
                oproj(c)
                if c == ng - 1:
                    wow_ref[...] = _pk(wobuf[0:DH, :])
                    refill(wo_cp, wobuf)

            def ev_qp(c):
                if c == ng:
                    wqw_ref[...] = _pk(wqbuf[0:D, :])
                    refill(wq_cp, wqbuf)
                assert not pre or c in lndone, c
                qproj(c)

            def ev_w5():
                v_cp(0).wait()
                x_cp(2).wait()
                for jj in range(nk):
                    vtr(0, jj)

            def ev_w6():
                for cp in (k_cp, v_cp, wq_cp):
                    cp(1).start()
                wo_cp(0).wait()
                x_cp(3).wait()
                wow_ref[...] = _pk(wobuf[0:DH, :])
                wo_cp(1).start()
                pin(wobuf, 2)
                for i in range(3):
                    f_cp(i).start()

            def ev_ln(pos):
                avail = [t for t in lnq if t < 3 * lnsub or pos >= w6]
                left = lambda c: max(len([1 for tt in lntimes if pos <= tt < min(qp(c), B)]), 1)
                cnt = 1
                for n_, t in enumerate(avail):
                    cnt = max(cnt, -(-(n_ + 4) // left(t // lnsub)))
                for p, sg in lnstage.items():
                    cnt = max(cnt, -(-(3 - sg) // left(p // lnsub)))
                for _ in range(cnt):
                    if avail or lnstage:
                        t = avail.pop(0) if avail else None
                        if t is not None:
                            lnq.remove(t)
                        tick(t)

            cmax = ng - 1 if post or pre else 2 * ng + 1
            ev = []
            for c in range(0, cmax + 1):
                for j in range(nk):
                    ev.append((p_qk(c, j), ev_qk, (c, j)))
                    ev.append((p_pv(c, j), ev_pv, (c, j)))
                if not (post and c == ng - 1):
                    ev.append((op(c), ev_op, (c,)))
                    ev.append((pr(c), oprep, (c,)))
                if c >= 1:
                    ev.append((qp(c), ev_qp, (c,)))
            if pre:
                lntimes = [t + 0.4 for t in range(w5, W)]
                ev += [(w5 - 0.01, ev_w5, ()), (w6 - 0.01, ev_w6, ())]
                ev += [(t, ev_ln, (t,)) for t in lntimes]
            if not post:
                ev += [(B - 0.001 if pre else gpos[k], gate_silu, (k,)) for k in range(GR // 16)]
            if post:
                ev += [(B, mod, ()), (int(B) + modpos + 0.4, mod_gu, ()),
                       (int(B) + dnpos + 0.45, mod_dn, ())]
            for t, f, a in sorted([e for e in ev if lo <= e[0] < hi], key=lambda e: e[0]):
                f(*a)

            if post:
                oprep(ng - 1)
                oproj(ng - 1, lastsub)
                for c in range(ng - 1):
                    o_cp(c).wait()
                for i in range(lastsub):
                    o_cp(ng - 1, i, lastsub).wait()
                return
            if pre:
                assert not lnq and not lnstage
            sh = 0 if pre else ng
            for i, c in enumerate(live_q):
                q_c[i] = _pk(qs[c + sh])
            for i, c in enumerate(live_mx):
                m_c[i] = maccs[c + sh]
            for i, c in enumerate(live_m):
                m_c[len(live_mx) + i] = ms[c + sh]
            for i, c in enumerate(live_o):
                l_c[i] = laccs[c + sh]
                o_c[i] = oaccs[c + sh]

        zero = zero_ref[0]
        if 'P' in parts:
            segment(0, 'pre', zero)

        def mid(h, carry):
            segment(h, 'mid', jnp.minimum(h, 0))
            return carry

        if 'M' in parts:
            lax.fori_loop(0, H - 1, mid, 0)
        if 'Q' in parts:
            segment(H - 1, 'post', zero)

    def kernel_w(zero_ref, *refs):
        return kernel(*refs[:10], zero_ref, *refs[10:])

    @jax.jit
    def fn(A_x, A_k_cache, A_v_cache, A_wq, A_wo, B_x, B_w_r, B_w_gate, B_w_up, B_w_down):
        x = A_x.reshape(S, D)
        k = A_k_cache.reshape(HH, S, DH)
        v = A_v_cache.reshape(HH, S, DH)
        wr = B_w_r
        hbm = pl.BlockSpec(memory_space=pl.ANY)
        V = pltpu.VMEM
        dma = pltpu.SemaphoreType.DMA
        out = pl.pallas_call(
            kernel_w,
            in_specs=[pl.BlockSpec(memory_space=pltpu.SMEM),
                      hbm, hbm, hbm, hbm, hbm, hbm, hbm, hbm, hbm],
            out_specs=hbm,
            out_shape=jax.ShapeDtypeStruct((S, D), bf16),
            scratch_shapes=[
                V((D,), bf16), V((16, D), f32), V((S, D), bf16), V((S + 16, DH), bf16), V((S + 16, DH), bf16), V((D + 16, DH), bf16), V((DH + 16, D), bf16),
                V((F, D), bf16), V((F, D), bf16), V((F, D), bf16),
                V((S // 2, D), u32), V((S // 2, D), u32), V((S // 128, 128), f32),
                V((S // 2, DH), u32), V((DH // 2, S), u32), V((D // 2, DH), u32), V((DH // 2, D), u32),
                V((len(live_mx) + len(live_m), 8, G), f32), V((len(live_o), 8, G), f32),
                V((len(live_o), DH, G), f32), V((len(live_q), G // 2, DH), u32),
                dma((nx,)), dma((4,)), dma((4,)), dma((ng - 1 + lastsub,)),
            ] + [V((S, G), f32)] * nbuf + [V((G // 2, DH), u32)] * nob + [V((G + 16, D), bf16)] * ng + [V((G, D), f32)] * ng,
            compiler_params=pltpu.CompilerParams(vmem_limit_bytes=100 * 1024 * 1024),
        )(jnp.zeros((1,), jnp.int32), x, k, v, A_wq, A_wo, wr, B_w_gate.T, B_w_up.T, B_w_down)
        return out.reshape(1, S, D)

    return fn


_impl = make(**{})


@jax.jit
def pallas_recurrent_scan__mha_block_cached__moe_arch_mod__prompt_kernel(A_x, A_k_cache, A_v_cache, A_wq, A_wo, B_x, B_w_r, B_w_gate, B_w_up, B_w_down):
    return _impl(A_x, A_k_cache, A_v_cache, A_wq, A_wo, B_x, B_w_r, B_w_gate, B_w_up, B_w_down)
```

```python
import jax
import jax.numpy as jnp
from jax import lax
import jax.experimental.pallas as pl
import jax.experimental.pallas.tpu as pltpu

S, D, HH, DH, F, C = 2048, 640, 32, 128, 1728, 8
LOG2E = 1.4426950408889634
NT = (((1,), (1,)), ((), ()))
f32 = jnp.float32
bf16 = jnp.bfloat16
u32 = jnp.uint32


def _rb(a):
    return a.astype(bf16).astype(f32)


def _gate(m, tok):
    return jnp.maximum(m, jnp.minimum(m, tok))


def _sigmoid(x):
    return 0.5 * jnp.tanh(0.5 * x) + 0.5


def _recip(d):
    r = pl.reciprocal(d, approx=True)
    r = r + r * (1.0 - d * r)
    return r + r * (1.0 - d * r)


def _pk(a):
    return pltpu.bitcast(a, u32)


def _upk(a):
    return pltpu.bitcast(a, bf16)


def make(G=256, KC=512, skew=1, lag=2, qpos=1.75, ppos=2.6, opos=10.5, nbuf=4, H=32, gates='lo', B=13.0,
         lnsub=4, modpos=3, dnpos=4, parts='PMQ', lntok=0, w5=-1, w6=4, lastsub=4, fp=0.25,
         fintok=2, gpos=(20.3, 24.3, 28.3, 32.3), nob=8, nz0=5, pinlag=1, oplag=1, gmode='none', tlag=3, opstep=1.0, tpos=16.1, carry_qt=True, crows=0, clag=2):
    ng = S // G
    nk = S // KC
    W = ng * nk
    ahead = nk + skew
    xsplit = (1, 1, 1, ng - 3)
    nx = len(xsplit)
    xoff = [sum(xsplit[:i]) for i in range(nx)]
    LR = G // lnsub
    GR = S // HH
    NF = -(-F // 128)

    p_qproj = lambda c: (c - 2) * nk + qpos
    p_qk = lambda c, j: c * nk + j - ahead
    p_pv = lambda c, j: c * nk + j + fp
    p_pr = lambda c: (c + 1) * nk + ppos
    p_op = lambda c: (c + 1) * nk + opos
    rng = range(-2, 2 * ng + 2)
    live_q = [c for c in rng if p_qproj(c) < B <= p_qk(c, nk - 1)]
    c0, j0 = min(((c, j) for c in rng for j in range(nk) if p_pv(c, j) >= B), key=lambda e: p_pv(*e))
    p_ex = lambda c, j: B - 0.0005 if crows and (c, j) == (c0, j0) else p_pv(c, j)
    live_mx = [c for c in rng if p_qk(c, 0) < B <= p_ex(c, 0)]
    live_m = [c for c in rng if p_ex(c, 0) < B <= p_pv(c, nk - 1)]
    live_l = [c for c in rng if p_ex(c, 0) < B <= p_pr(c)]
    live_o = [c for c in rng if p_pv(c, 0) < B <= p_pr(c)]

    def kernel(x_hbm, k_hbm, v_hbm, wq_hbm, wo_hbm, wr_hbm, wg_hbm, wu_hbm, wd_hbm, o_hbm,
               zero_ref, wr_ref, wrf_ref, x_ref, kbuf, vbuf, wqbuf, wobuf, wgu_ref, wt_ref, wd_ref,
               xn_ref, g_ref, r_ref, kw_ref, vt_ref, wqw_ref, wow_ref,
               m_c, l_c, o_c, q_c, p_c,
               xsem, hsem, fsem, osem, *rest):
        s_refs, rest = rest[:nbuf], rest[nbuf:]
        o_refs, ob_refs, acc_refs = rest[:nob], rest[nob:nob + ng], rest[nob + ng:]

        def x_cp(i):
            rows = pl.ds(xoff[i] * G, xsplit[i] * G)
            return pltpu.make_async_copy(x_hbm.at[rows, :], x_ref.at[rows, :], xsem.at[i])

        def k_cp(h):
            return pltpu.make_async_copy(k_hbm.at[h], kbuf.at[0:S, :], hsem.at[0])

        def v_cp(h):
            return pltpu.make_async_copy(v_hbm.at[h], vbuf.at[0:S, :], hsem.at[1])

        def wq_cp(h):
            col = h * DH if isinstance(h, int) else pl.multiple_of(h * DH, DH)
            return pltpu.make_async_copy(wq_hbm.at[:, pl.ds(col, DH)], wqbuf.at[0:D, :], hsem.at[2])

        def wo_cp(h):
            row = h * DH if isinstance(h, int) else pl.multiple_of(h * DH, DH)
            return pltpu.make_async_copy(wo_hbm.at[pl.ds(row, DH), :], wobuf.at[0:DH, :], hsem.at[3])

        def f_cp(i):
            src = (wg_hbm, wu_hbm, wd_hbm, wr_hbm)[i]
            dst = (wgu_ref.at[0:F, :], wgu_ref.at[F:2 * F, :], wd_ref, wr_ref)[i]
            return pltpu.make_async_copy(src, dst, fsem.at[i])

        def o_cp(c, i=0, nsub=1):
            n = G // nsub
            return pltpu.make_async_copy(ob_refs[c].at[i * n:(i + 1) * n, :], o_hbm.at[pl.ds(c * G + i * n, n), :],
                                         osem.at[c + i])

        def grow(c):
            return pl.ds((c % ng) * G, G)

        def hrow(c):
            return pl.ds((c % ng) * (G // 2), G // 2)

        def segment(h, mode, zero):
            pre, post = mode == 'pre', mode == 'post'
            qs, qts, maccs, ms, laccs, oaccs, ps = {}, {}, {}, {}, {}, {}, {}
            hist = {}
            lastm = [None]
            extra = []

            def after(tok):
                if tok is None:
                    return 0
                return pltpu.bitcast(tok, jnp.int32)[0, 0] & zero

            def pin(ref, lagn, val=None):
                spare = pl.ds(pl.multiple_of(zero + (ref.shape[0] - 16), 16), 16)
                ref[spare, 0:128] = jnp.zeros((16, 128), bf16) if val is None else val
                t = pltpu.bitcast(ref[spare, 0:128], f32)
                extra.append((len(hist) + lagn, jnp.concatenate([t] * (G // 128), axis=1)))

            def refill(cp, ref):
                @pl.when(h + 2 < H)
                def _():
                    cp(h + 2).start()
                pin(ref, pinlag)

            lane = lax.broadcasted_iota(jnp.int32, (8, 128), 1)

            lnst = {}

            def ln_a(t):
                xs = []
                for r in range(t * LR, (t + 1) * LR, 16):
                    x16 = x_ref[r:r + 16, :].astype(f32)
                    xs += [x16[:8], x16[8:]]
                means = [jnp.sum(x, axis=-1, keepdims=True) * (1.0 / D) for x in xs]
                lnst[t] = dict(xs=xs, means=means)
                return means[-1]

            def ln_b(t):
                st = lnst[t]
                ssq = jnp.zeros((8, 128), f32)
                dm = jnp.zeros((8, 128), f32)
                ds = []
                for k, (x, mean) in enumerate(zip(st['xs'], st['means'])):
                    mk = _rb(mean)
                    d = x - mk
                    ds.append(d)
                    ssq = jnp.where(lane == k, jnp.sum(d * d, axis=-1, keepdims=True), ssq)
                    dm = jnp.where(lane == k, mean - mk, dm)
                st['d'] = [jnp.concatenate(ds[k:k + 2], axis=0).astype(bf16) for k in range(0, LR // 8, 2)]
                var = jnp.maximum(ssq * (1.0 / D) - dm * dm, 0.0)
                st['inv'] = 1.0 / _rb(jnp.sqrt(_rb(_rb(var) + _rb(f32(1e-5)))))
                return st['inv']

            def ln_b2(t):
                st = lnst[t]
                st['invs'] = [jnp.sum(jnp.where(lane == k, st['inv'], 0.0), axis=-1, keepdims=True)
                              for k in range(LR // 8)]
                return st['invs'][-1]

            def ln_c(t):
                st = lnst.pop(t)
                for k in range(0, LR // 8, 2):
                    d = st['d'][k // 2].astype(f32)
                    xn = jnp.concatenate([d[:8] * st['invs'][k], d[8:] * st['invs'][k + 1]], axis=0)
                    r = t * LR + k * 8
                    xn_ref[r // 2:r // 2 + 8, :] = _pk(xn.astype(bf16))
                if (t + 1) % lnsub == 0:
                    lndone.add(t // lnsub)
                return xn[8:, D - 128:]

            lnstage = {}

            def tick(t, tok=True):
                toks = []
                for p in sorted(lnstage):
                    toks.append((ln_b, ln_b2, ln_c)[lnstage[p]](p))
                    lnstage[p] += 1
                    if lnstage[p] == 3:
                        del lnstage[p]
                if t is not None:
                    toks.append(ln_a(t))
                    lnstage[t] = 0
                if tok and lntok:
                    for tk in toks:
                        extra.append((len(hist) + lntok, jnp.broadcast_to(
                            tk if tk.shape[1] == 1 else jnp.concatenate([tk] * (G // 128), axis=1), (8, G))))

            def qproj(c):
                q = jnp.dot(_upk(xn_ref[hrow(c), :]), _upk(wqw_ref[...]), preferred_element_type=f32)
                qs[c] = (q * (DH ** -0.5 * LOG2E)).astype(bf16)

            def qk(c, j):
                kk = _upk(kw_ref[j * KC // 2:(j + 1) * KC // 2, :])
                if c in qts:
                    st = jnp.dot(kk, qts[c], preferred_element_type=f32)
                else:
                    st = lax.dot_general(kk, qs[c], NT, preferred_element_type=f32)
                off = pl.multiple_of(zero + j * KC, KC)
                s_refs[c % nbuf][pl.ds(off, KC), :] = st
                mm = jnp.max(st.reshape(KC // 8, 8, G), axis=0)
                maccs[c] = mm if j == 0 else jnp.maximum(maccs[c], mm)
                lastm[0] = maccs[c]

            def kcopy(hh, j):
                kw_ref[j * KC // 2:(j + 1) * KC // 2, :] = _pk(kbuf[j * KC:(j + 1) * KC, :])

            def vtr(hh, j):
                vt_ref[:, j * KC:(j + 1) * KC] = _pk(vbuf[j * KC:(j + 1) * KC, :].T)

            def ex(c, j, r0=0, r1=KC, lg=None):
                if j == 0 and r0 == 0:
                    ms[c] = jnp.broadcast_to(jnp.max(maccs[c], axis=0, keepdims=True), (8, G))
                m = ms[c]
                if lg is None:
                    lg = tlag if post and c * nk + j > W - ahead else lag
                for tok in hist.get(c * nk + j - lg, ()):
                    m = _gate(m, tok)
                for e in [e for e in extra if e[0] <= len(hist)]:
                    m = _gate(m, e[1])
                extra[:] = [e for e in extra if e[0] > len(hist)]
                p = jnp.exp2(s_refs[c % nbuf][j * KC + r0:j * KC + r1, :].reshape((r1 - r0) // 8, 8, G) - m[None])
                ll = jnp.sum(p, axis=0)
                laccs[c] = ll if j == 0 and r0 == 0 else laccs[c] + ll
                return p.reshape(r1 - r0, G).astype(bf16)

            def pv(c, j):
                r0 = 0
                if (c, j) in ps:
                    r0 = crows
                    oo = jnp.dot(_upk(vt_ref[:, j * KC:j * KC + r0]), ps.pop((c, j)), preferred_element_type=f32)
                    oaccs[c] = oo if j == 0 else oaccs[c] + oo
                oo = jnp.dot(_upk(vt_ref[:, j * KC + r0:(j + 1) * KC]), ex(c, j, r0), preferred_element_type=f32)
                oaccs[c] = oo if j == 0 and r0 == 0 else oaccs[c] + oo
                toks = []
                if 'm' in gates and lastm[0] is not None:
                    toks.append(lastm[0])
                if 'l' in gates:
                    toks.append(laccs[c])
                if 'o' in gates:
                    toks.append(oaccs[c][DH - 8:, :])
                hist[c * nk + j] = toks

            def oprep(c):
                l = jnp.sum(laccs[c], axis=0, keepdims=True)
                o_refs[c % nob][...] = _pk((oaccs[c] * (1.0 / l)).T.astype(bf16))

            def oproj(c, nsub=1):
                n = G // nsub
                for i in range(nsub):
                    rows = pl.ds(i * n, n)
                    y = jnp.dot(_upk(o_refs[c % nob][i * n // 2:(i + 1) * n // 2, :]), _upk(wow_ref[...]),
                                preferred_element_type=f32)
                    if pre:
                        acc_refs[c][rows, :] = y
                    elif not post:
                        acc_refs[c % ng][rows, :] += y
                    else:
                        for r in range(i * n, (i + 1) * n, 16):
                            g = _upk(g_ref[(c * G + r) // 2:(c * G + r) // 2 + 8, :]).astype(f32)
                            sv = acc_refs[c][r:r + 16, :] + y[r - i * n:r - i * n + 16]
                            o = (x_ref[c * G + r:c * G + r + 16, :].astype(f32) + sv * g).astype(bf16)
                            ob_refs[c][r:r + 16, :] = o
                        o_cp(c, i, nsub).start()
                if post and nsub == 1 and fintok:
                    pin(ob_refs[c], fintok, o[:, D - 128:])

            md = {}

            def mod():
                r = _rb(r_ref[...]) + 0.0
                i0 = lax.broadcasted_iota(jnp.int32, r.shape, 0)
                ids = ((i0 >> 3) * 128 + lax.broadcasted_iota(jnp.int32, r.shape, 1)) * 8 + (i0 & 7)
                bits = pltpu.bitcast(r, jnp.int32)
                hi = jnp.where(bits < 0, bits ^ 0x7FFF0000, bits)
                hi = jnp.where(r != r, jnp.int32(-2 ** 31), hi)
                key = hi | (S - ids)
                rid = lax.broadcasted_iota(jnp.int32, (C, 1), 0)
                ksel = jnp.zeros((C, 1), jnp.int32)
                idxs, rows = [], []
                for j in range(C):
                    mx = jnp.max(key, keepdims=True)
                    key = jnp.where(key == mx, jnp.int32(-2 ** 31), key)
                    ksel = jnp.where(rid == j, mx, ksel)
                    am = S - (mx[0, 0] & 0xFFFF)
                    idxs.append(am)
                    w = xn_ref[pl.ds(lax.shift_right_logical(am, 1), 1), :]
                    sh = ((am & 1) * 16).astype(u32)
                    rows.append(lax.shift_left(lax.shift_right_logical(w, sh), u32(16)))
                xs = pltpu.bitcast(jnp.concatenate(rows, axis=0), f32)
                xsb = xs.astype(bf16)
                ksel = ksel & jnp.int32(-65536)
                rsel = pltpu.bitcast(jnp.broadcast_to(jnp.where(ksel < 0, ksel ^ 0x7FFF0000, ksel), (C, 128)), f32)[:, 0:1]
                md.update(xs=xs, xsb=xsb, idxs=idxs, rsel=rsel)

            def mod_gu():
                xsb = md['xsb']
                a, u = [jnp.dot(xsb, jnp.concatenate([_upk(wt_ref[mt * NF + t]) for t in range(NF)], axis=1),
                                preferred_element_type=f32) for mt in (0, 1)]
                col = lax.broadcasted_iota(jnp.int32, a.shape, 1)
                dup = jnp.logical_and(col >= (NF - 1) * 128, col < (NF - 1) * 128 + (NF * 128 - F))
                md['hh'] = jnp.where(dup, 0.0, a * _sigmoid(a) * u).astype(bf16)

            def mod_dn():
                xs, idxs, rsel = md['xs'], md['idxs'], md['rsel']
                n0 = (NF - 1) * 128
                y = (jnp.dot(md['hh'][:, :n0], wd_ref[0:n0, :], preferred_element_type=f32)
                     + jnp.dot(md['hh'][:, n0:], wd_ref[F - 128:F, :], preferred_element_type=f32))
                zz = xs + y * _sigmoid(rsel)
                hz = _rb(zz) * 0.5
                zb = lax.shift_right_logical(pltpu.bitcast(_rb(hz * jnp.tanh(hz) + hz), u32), u32(16))
                for j in range(C):
                    row = pl.ds(lax.shift_right_logical(idxs[j], 1), 1)
                    sh = ((idxs[j] & 1) * 16).astype(u32)
                    keep = lax.shift_left(u32(0xFFFF), u32(16) - sh)
                    g_ref[row, :] = (g_ref[row, :] & keep) | lax.shift_left(zb[j:j + 1, :], sh)

            def wtr():
                t = h - 1
                real = jnp.logical_and(t >= 0, t < 2 * NF)
                mt = (t >= NF).astype(jnp.int32)
                src = jnp.where(real, mt * F + jnp.minimum((t - mt * NF) * 128, F - 128), 2 * F)
                blk = wgu_ref[pl.ds(pl.multiple_of(src, 64), 128), :]
                wt_ref[jnp.where(real, t, 2 * NF)] = _pk(blk.T)

            def gate_silu(k):
                if pre:
                    rg = (H - 1) * (GR // 8) + 2 * k
                    rows = pl.ds(rg * 4, 8)
                else:
                    rg = h * (GR // 8) + 2 * k
                    rows = pl.ds(pl.multiple_of(rg * 4 + (after(hist[max(hist)][-1][:, :128]) if gmode == 'after' else 0), 8), 8)
                xp = xn_ref[rows, :]
                if gmode == 'or' and not pre:
                    zz = pltpu.bitcast(hist[max(hist)][-1][:, :128], u32) & zero.astype(u32)
                    xp = xp | jnp.concatenate([zz] * (D // 128), axis=1)
                xn = _upk(xp).astype(f32)
                hz = xn * 0.5
                g_ref[rows, :] = _pk((hz * jnp.tanh(hz) + hz).astype(bf16))
                xw = xn * wrf_ref[...]
                rr = [jnp.sum(xw[kk * 8:kk * 8 + 8], axis=-1, keepdims=True) for kk in (0, 1)]
                for v in range(S // 1024):
                    r = r_ref[v * 8:v * 8 + 8, :]
                    for kk in (0, 1):
                        r = jnp.where(lane == rg + (kk - v * 128), rr[kk], r)
                    r_ref[v * 8:v * 8 + 8, :] = r

            lnq = []
            lndone = set()
            if pre:
                x_cp(0).start()
                f_cp(3).start()
                wq_cp(0).start()
                k_cp(0).start()
                x_cp(1).start()
                zq = [c for c in range(ng) if p_op(c) >= B]
                for c in zq[:nz0]:
                    acc_refs[c][...] = jnp.zeros((G, D), f32)
                x_cp(0).wait()
                f_cp(3).wait()
                wrf_ref[...] = jnp.broadcast_to(wr_ref[...].astype(f32).reshape(1, D), (16, D))
                r_ref[...] = jnp.zeros(r_ref.shape, f32)
                wgu_ref[2 * F:, :] = jnp.zeros((128, D), bf16)
                v_cp(0).start()
                x_cp(2).start()
                for t in range(lnsub):
                    tick(t, False)
                while lnstage:
                    tick(None, False)
                wo_cp(0).start()
                wq_cp(0).wait()
                x_cp(3).start()
                wqw_ref[...] = _pk(wqbuf[0:D, :])
                qproj(0)
                for c in zq[nz0:]:
                    acc_refs[c][...] = jnp.zeros((G, D), f32)
                k_cp(0).wait()
                x_cp(1).wait()
                for j in range(nk):
                    kcopy(0, j)
                for t in range(lnsub, 2 * lnsub):
                    tick(t, False)
                while lnstage:
                    tick(None, False)
                lnq = list(range(2 * lnsub, ng * lnsub))
                lo, hi = -ahead, B
            elif post:
                f_cp(2).wait()
                lo, hi = B, W
            else:
                for cp in (k_cp, v_cp, wq_cp, wo_cp):
                    cp(h + 1).wait()

                @pl.when(h == 1)
                def _():
                    f_cp(0).wait()
                    f_cp(1).wait()
                lo, hi = B, B + W

            if not pre:
                for i, c in enumerate(live_q):
                    (qts if carry_qt else qs)[c] = _upk(q_c[i])
                if crows:
                    ps[c0, j0] = _upk(p_c[...])
                for i, c in enumerate(live_mx):
                    maccs[c] = m_c[i]
                for i, c in enumerate(live_m):
                    ms[c] = m_c[len(live_mx) + i]
                for i, c in enumerate(live_l):
                    laccs[c] = l_c[i]
                for i, c in enumerate(live_o):
                    oaccs[c] = o_c[i]

            assert p_op(0) >= B or not post
            pr = lambda c: max(B, (c + 1) * nk + 0.3) if post and p_pr(c) >= B else p_pr(c)
            if post:
                op = lambda c: max(pr(c) + oplag, int(B) + dnpos + 1.5 + int(c * opstep))
            else:
                op = lambda c: max(p_op(c), w6 + 0.5) if pre else p_op(c)
            qp = lambda c: min(max(p_qproj(c), w6 + 0.75), p_qk(c, 0) - 0.25) if pre and c >= 3 else p_qproj(c)

            def ev_qk(c, j):
                qk(c, j)
                if c == ng - 1 and not post:
                    kcopy(h + 1, j)
                    if j == nk - 1:
                        refill(k_cp, kbuf)

            def ev_pv(c, j):
                pv(c, j)
                if c == ng - 1 and not post:
                    vtr(h + 1, j)
                    if j == nk - 1:
                        refill(v_cp, vbuf)

            def ev_op(c):
                oproj(c)
                if c == ng - 1:
                    wow_ref[...] = _pk(wobuf[0:DH, :])
                    refill(wo_cp, wobuf)

            def ev_qp(c):
                if c == ng:
                    wqw_ref[...] = _pk(wqbuf[0:D, :])
                    refill(wq_cp, wqbuf)
                assert not pre or c in lndone, c
                qproj(c)

            def ev_w5():
                v_cp(0).wait()
                x_cp(2).wait()
                wo_cp(0).wait()
                for jj in range(nk):
                    vtr(0, jj)
                wow_ref[...] = _pk(wobuf[0:DH, :])

            def ev_w6():
                for cp in (k_cp, v_cp, wq_cp, wo_cp):
                    cp(1).start()
                x_cp(3).wait()
                for i in range(3):
                    f_cp(i).start()

            def ev_ln(pos):
                avail = [t for t in lnq if t < 3 * lnsub or pos >= w6]
                left = lambda c: max(len([1 for tt in lntimes if pos <= tt < min(qp(c), B)]), 1)
                cnt = 1
                for n_, t in enumerate(avail):
                    cnt = max(cnt, -(-(n_ + 4) // left(t // lnsub)))
                for p, sg in lnstage.items():
                    cnt = max(cnt, -(-(3 - sg) // left(p // lnsub)))
                for _ in range(cnt):
                    if avail or lnstage:
                        t = avail.pop(0) if avail else None
                        if t is not None:
                            lnq.remove(t)
                        tick(t)

            cmax = ng - 1 if post or pre else 2 * ng + 1
            ev = []
            for c in range(0, cmax + 1):
                for j in range(nk):
                    ev.append((p_qk(c, j), ev_qk, (c, j)))
                    ev.append((p_pv(c, j), ev_pv, (c, j)))
                if not (post and c == ng - 1):
                    ev.append((op(c), ev_op, (c,)))
                    ev.append((pr(c), oprep, (c,)))
                if c >= 1:
                    ev.append((qp(c), ev_qp, (c,)))
            if pre:
                lntimes = [t + 0.4 for t in range(w5, W)]
                ev += [(w5 - 0.01, ev_w5, ()), (w6 - 0.01, ev_w6, ())]
                ev += [(t, ev_ln, (t,)) for t in lntimes]
            if not post:
                ev += [(B - 0.001 if pre else gpos[k], gate_silu, (k,)) for k in range(GR // 16)]
            if not pre and not post:
                ev.append((tpos, wtr, ()))
            if post:
                ev += [(B, mod, ()), (int(B) + modpos + 0.4, mod_gu, ()),
                       (int(B) + dnpos + 0.45, mod_dn, ())]
            for t, f, a in sorted([e for e in ev if lo <= e[0] < hi], key=lambda e: e[0]):
                f(*a)

            if post:
                oprep(ng - 1)
                oproj(ng - 1, lastsub)
                for c in range(ng - 1):
                    o_cp(c).wait()
                for i in range(lastsub):
                    o_cp(ng - 1, i, lastsub).wait()
                return
            if pre:
                assert not lnq and not lnstage
            sh = 0 if pre else ng
            if crows:
                p_c[...] = _pk(ex(c0 + sh, j0, 0, crows, clag))
            for i, c in enumerate(live_q):
                q_c[i] = _pk(qs[c + sh].T if carry_qt else qs[c + sh])
            for i, c in enumerate(live_mx):
                m_c[i] = maccs[c + sh]
            for i, c in enumerate(live_m):
                m_c[len(live_mx) + i] = ms[c + sh]
            for i, c in enumerate(live_l):
                l_c[i] = laccs[c + sh]
            for i, c in enumerate(live_o):
                o_c[i] = oaccs[c + sh]

        zero = zero_ref[0]
        if 'P' in parts:
            segment(0, 'pre', zero)

        def mid(h, carry):
            segment(h, 'mid', jnp.minimum(h, 0))
            return carry

        if 'M' in parts:
            lax.fori_loop(0, H - 1, mid, 0)
        if 'Q' in parts:
            segment(H - 1, 'post', zero)

    def kernel_w(zero_ref, *refs):
        return kernel(*refs[:10], zero_ref, *refs[10:])

    @jax.jit
    def fn(A_x, A_k_cache, A_v_cache, A_wq, A_wo, B_x, B_w_r, B_w_gate, B_w_up, B_w_down):
        x = A_x.reshape(S, D)
        k = A_k_cache.reshape(HH, S, DH)
        v = A_v_cache.reshape(HH, S, DH)
        wr = B_w_r
        hbm = pl.BlockSpec(memory_space=pl.ANY)
        V = pltpu.VMEM
        dma = pltpu.SemaphoreType.DMA
        out = pl.pallas_call(
            kernel_w,
            in_specs=[pl.BlockSpec(memory_space=pltpu.SMEM),
                      hbm, hbm, hbm, hbm, hbm, hbm, hbm, hbm, hbm],
            out_specs=hbm,
            out_shape=jax.ShapeDtypeStruct((S, D), bf16),
            scratch_shapes=[
                V((D,), bf16), V((16, D), f32), V((S, D), bf16), V((S + 16, DH), bf16), V((S + 16, DH), bf16), V((D + 16, DH), bf16), V((DH + 16, D), bf16),
                V((2 * F + 128, D), bf16), V((2 * NF + 1, D // 2, 128), u32), V((F, D), bf16),
                V((S // 2, D), u32), V((S // 2, D), u32), V((S // 128, 128), f32),
                V((S // 2, DH), u32), V((DH // 2, S), u32), V((D // 2, DH), u32), V((DH // 2, D), u32),
                V((len(live_mx) + len(live_m), 8, G), f32), V((len(live_l), 8, G), f32),
                V((max(len(live_o), 1), DH, G), f32),
                V((len(live_q), DH // 2, G) if carry_qt else (len(live_q), G // 2, DH), u32), V((max(crows, 16) // 2, G), u32),
                dma((nx,)), dma((4,)), dma((4,)), dma((ng - 1 + lastsub,)),
            ] + [V((S, G), f32)] * nbuf + [V((G // 2, DH), u32)] * nob + [V((G + 16, D), bf16)] * ng + [V((G, D), f32)] * ng,
            compiler_params=pltpu.CompilerParams(vmem_limit_bytes=100 * 1024 * 1024),
        )(jnp.zeros((1,), jnp.int32), x, k, v, A_wq, A_wo, wr, B_w_gate.T, B_w_up.T, B_w_down)
        return out.reshape(1, S, D)

    return fn


_impl = make(**{})


@jax.jit
def pallas_recurrent_scan__mha_block_cached__moe_arch_mod__prompt_kernel(A_x, A_k_cache, A_v_cache, A_wq, A_wo, B_x, B_w_r, B_w_gate, B_w_up, B_w_down):
    return _impl(A_x, A_k_cache, A_v_cache, A_wq, A_wo, B_x, B_w_r, B_w_gate, B_w_up, B_w_down)
```

```python
import jax
import jax.numpy as jnp
from jax import lax
import jax.experimental.pallas as pl
import jax.experimental.pallas.tpu as pltpu

S, D, H, DH, F, C = 2048, 640, 32, 128, 1728, 8
LOG2E = 1.4426950408889634
NT = (((1,), (1,)), ((), ()))
f32 = jnp.float32
bf16 = jnp.bfloat16
u32 = jnp.uint32

G = 256
KC = 512
NG = S // G
NK = S // KC
W = NG * NK
AHEAD = NK + 1
B = 13
NSBUF = 4
LAG, TAIL_LAG = 2, 4
LNSUB = 4
LR = G // LNSUB
GR = S // H
NF = -(-F // 128)
XSPLIT = (1, 1, 1, NG - 3)
XOFF = tuple(sum(XSPLIT[:i]) for i in range(len(XSPLIT)))
W5, W6 = -1, 5
LASTSUB = 8

p_qproj = lambda c: (c - 2) * NK + 1.75
p_qk = lambda c, j: c * NK + j - AHEAD
p_pv = lambda c, j: c * NK + j + 0.25
p_prep = lambda c: (c + 1) * NK + 2.6
p_oproj = lambda c: (c + 1) * NK + 10.5
_rng = range(-2, 2 * NG + 2)
LIVE_Q = [c for c in _rng if p_qproj(c) < B <= p_qk(c, NK - 1)]
LIVE_MX = [c for c in _rng if p_qk(c, 0) < B <= p_pv(c, 0)]
LIVE_M = [c for c in _rng if p_pv(c, 0) < B <= p_pv(c, NK - 1)]
LIVE_O = [c for c in _rng if p_pv(c, 0) < B <= p_prep(c)]
assert p_oproj(0) >= B


def _rb(a):
    return a.astype(bf16).astype(f32)


def _gate(m, tok):
    return jnp.maximum(m, jnp.minimum(m, tok))


def _sigmoid(x):
    return 0.5 * jnp.tanh(0.5 * x) + 0.5


def _silu(x):
    hx = x * 0.5
    return hx * jnp.tanh(hx) + hx


def _pk(a):
    return pltpu.bitcast(a, u32)


def _upk(a):
    return pltpu.bitcast(a, bf16)


def _kernel(zero_ref, x_hbm, k_hbm, v_hbm, wq_hbm, wo_hbm, wr_hbm, wg_hbm, wu_hbm, wd_hbm, o_hbm,
            wr_ref, wrf_ref, x_ref, kbuf, vbuf, wqbuf, wobuf, wgu_ref, wt_ref, wd_ref,
            xn_ref, g_ref, r_ref, kw_ref, vt_ref, wqw_ref, wow_ref,
            m_c, l_c, o_c, q_c,
            xsem, hsem, fsem, osem, *rest):
    s_refs, rest = rest[:NSBUF], rest[NSBUF:]
    o_refs, ob_refs, acc_refs = rest[:NG], rest[NG:2 * NG], rest[2 * NG:]

    def x_cp(i):
        rows = pl.ds(XOFF[i] * G, XSPLIT[i] * G)
        return pltpu.make_async_copy(x_hbm.at[rows, :], x_ref.at[rows, :], xsem.at[i])

    def k_cp(h):
        return pltpu.make_async_copy(k_hbm.at[h], kbuf.at[0:S, :], hsem.at[0])

    def v_cp(h):
        return pltpu.make_async_copy(v_hbm.at[h], vbuf.at[0:S, :], hsem.at[1])

    def wq_cp(h):
        col = h * DH if isinstance(h, int) else pl.multiple_of(h * DH, DH)
        return pltpu.make_async_copy(wq_hbm.at[:, pl.ds(col, DH)], wqbuf.at[0:D, :], hsem.at[2])

    def wo_cp(h):
        row = h * DH if isinstance(h, int) else pl.multiple_of(h * DH, DH)
        return pltpu.make_async_copy(wo_hbm.at[pl.ds(row, DH), :], wobuf.at[0:DH, :], hsem.at[3])

    def f_cp(i):
        src = (wg_hbm, wu_hbm, wd_hbm, wr_hbm)[i]
        dst = (wgu_ref.at[0:F, :], wgu_ref.at[F:2 * F, :], wd_ref, wr_ref)[i]
        return pltpu.make_async_copy(src, dst, fsem.at[i])

    def o_cp(c, i=0, nsub=1):
        n = G // nsub
        return pltpu.make_async_copy(ob_refs[c].at[i * n:(i + 1) * n, :], o_hbm.at[pl.ds(c * G + i * n, n), :],
                                     osem.at[c + i])

    def segment(h, mode, zero):
        pre, post = mode == 'pre', mode == 'post'
        qs, qts, maccs, ms, laccs, oaccs = {}, {}, {}, {}, {}, {}
        hist = {}
        extra = []

        def pin(ref, lagn):
            spare = pl.ds(pl.multiple_of(zero + (ref.shape[0] - 16), 16), 16)
            ref[spare, 0:128] = jnp.zeros((16, 128), bf16)
            t = pltpu.bitcast(ref[spare, 0:128], f32)
            extra.append((len(hist) + lagn, jnp.concatenate([t] * (G // 128), axis=1)))

        def refill(cp, ref):
            @pl.when(h + 2 < H)
            def _():
                cp(h + 2).start()
            pin(ref, 1)

        lane = lax.broadcasted_iota(jnp.int32, (8, 128), 1)

        lnst, lnstage, lndone = {}, {}, set()

        def ln_a(t):
            xs = []
            for r in range(t * LR, (t + 1) * LR, 16):
                x16 = x_ref[r:r + 16, :].astype(f32)
                xs += [x16[:8], x16[8:]]
            lnst[t] = dict(xs=xs, means=[jnp.sum(x, axis=-1, keepdims=True) * (1.0 / D) for x in xs])

        def ln_b(t):
            st = lnst[t]
            ssq = jnp.zeros((8, 128), f32)
            dm = jnp.zeros((8, 128), f32)
            ds = []
            for k, (x, mean) in enumerate(zip(st['xs'], st['means'])):
                mk = _rb(mean)
                d = x - mk
                ds.append(d)
                ssq = jnp.where(lane == k, jnp.sum(d * d, axis=-1, keepdims=True), ssq)
                dm = jnp.where(lane == k, mean - mk, dm)
            st['d'] = [jnp.concatenate(ds[k:k + 2], axis=0).astype(bf16) for k in range(0, LR // 8, 2)]
            var = jnp.maximum(ssq * (1.0 / D) - dm * dm, 0.0)
            st['inv'] = 1.0 / _rb(jnp.sqrt(_rb(_rb(var) + _rb(f32(1e-5)))))

        def ln_b2(t):
            st = lnst[t]
            st['invs'] = [jnp.sum(jnp.where(lane == k, st['inv'], 0.0), axis=-1, keepdims=True)
                          for k in range(LR // 8)]

        def ln_c(t):
            st = lnst.pop(t)
            for k in range(0, LR // 8, 2):
                d = st['d'][k // 2].astype(f32)
                xn = jnp.concatenate([d[:8] * st['invs'][k], d[8:] * st['invs'][k + 1]], axis=0)
                r = t * LR + k * 8
                xn_ref[r // 2:r // 2 + 8, :] = _pk(xn.astype(bf16))
            if (t + 1) % LNSUB == 0:
                lndone.add(t // LNSUB)

        def tick(t):
            for p in sorted(lnstage):
                (ln_b, ln_b2, ln_c)[lnstage[p]](p)
                lnstage[p] += 1
                if lnstage[p] == 3:
                    del lnstage[p]
            if t is not None:
                ln_a(t)
                lnstage[t] = 0

        def ln_group(c):
            for t in range(c * LNSUB, (c + 1) * LNSUB):
                tick(t)
            while lnstage:
                tick(None)

        def qproj(c):
            r0 = (c % NG) * (G // 2)
            q = jnp.dot(_upk(xn_ref[r0:r0 + G // 2, :]), _upk(wqw_ref[...]), preferred_element_type=f32)
            qs[c] = (q * (DH ** -0.5 * LOG2E)).astype(bf16)

        def qk(c, j):
            kk = _upk(kw_ref[j * KC // 2:(j + 1) * KC // 2, :])
            if c in qts:
                st = jnp.dot(kk, qts[c], preferred_element_type=f32)
            else:
                st = lax.dot_general(kk, qs[c], NT, preferred_element_type=f32)
            off = pl.multiple_of(zero + j * KC, KC)
            s_refs[c % NSBUF][pl.ds(off, KC), :] = st
            mm = jnp.max(st.reshape(KC // 8, 8, G), axis=0)
            maccs[c] = mm if j == 0 else jnp.maximum(maccs[c], mm)

        def kcopy(j):
            kw_ref[j * KC // 2:(j + 1) * KC // 2, :] = _pk(kbuf[j * KC:(j + 1) * KC, :])

        def vtr(j):
            vt_ref[:, j * KC:(j + 1) * KC] = _pk(vbuf[j * KC:(j + 1) * KC, :].T)

        def pv(c, j):
            if j == 0:
                ms[c] = jnp.broadcast_to(jnp.max(maccs[c], axis=0, keepdims=True), (8, G))
            m = ms[c]
            n = c * NK + j
            for tok in hist.get(n - (TAIL_LAG if post and n > W - AHEAD else LAG), ()):
                m = _gate(m, tok)
            for e in [e for e in extra if e[0] <= len(hist)]:
                m = _gate(m, e[1])
            extra[:] = [e for e in extra if e[0] > len(hist)]
            vt = _upk(vt_ref[:, j * KC:(j + 1) * KC])
            p = jnp.exp2(s_refs[c % NSBUF][j * KC:(j + 1) * KC, :].reshape(KC // 8, 8, G) - m[None])
            ll = jnp.sum(p, axis=0)
            laccs[c] = ll if j == 0 else laccs[c] + ll
            oo = jnp.dot(vt, p.reshape(KC, G).astype(bf16), preferred_element_type=f32)
            oaccs[c] = oo if j == 0 else oaccs[c] + oo
            hist[n] = [laccs[c], oaccs[c][DH - 8:, :]]

        def oprep(c):
            l = jnp.sum(laccs[c], axis=0, keepdims=True)
            o_refs[c % NG][...] = _pk((oaccs[c] * (1.0 / l)).T.astype(bf16))

        def oproj(c, nsub=1):
            n = G // nsub
            for i in range(nsub):
                y = jnp.dot(_upk(o_refs[c % NG][i * n // 2:(i + 1) * n // 2, :]), _upk(wow_ref[...]),
                            preferred_element_type=f32)
                if not post:
                    acc_refs[c % NG][i * n:(i + 1) * n, :] += y
                else:
                    for r in range(i * n, (i + 1) * n, 16):
                        g = _upk(g_ref[(c * G + r) // 2:(c * G + r) // 2 + 8, :]).astype(f32)
                        sv = acc_refs[c][r:r + 16, :] + y[r - i * n:r - i * n + 16]
                        ob_refs[c][r:r + 16, :] = (x_ref[c * G + r:c * G + r + 16, :].astype(f32) + sv * g).astype(bf16)
                    o_cp(c, i, nsub).start()
            if post and nsub == 1:
                pin(ob_refs[c], 2)

        md = {}

        def mod_select():
            r = _rb(r_ref[...]) + 0.0
            i0 = lax.broadcasted_iota(jnp.int32, r.shape, 0)
            ids = ((i0 >> 3) * 128 + lax.broadcasted_iota(jnp.int32, r.shape, 1)) * 8 + (i0 & 7)
            bits = pltpu.bitcast(r, jnp.int32)
            hi = jnp.where(bits < 0, bits ^ 0x7FFF0000, bits)
            hi = jnp.where(r != r, jnp.int32(-2 ** 31), hi)
            key = hi | (S - ids)
            rid = lax.broadcasted_iota(jnp.int32, (C, 1), 0)
            ksel = jnp.zeros((C, 1), jnp.int32)
            idxs, rows = [], []
            for j in range(C):
                mx = jnp.max(key, keepdims=True)
                key = jnp.where(key == mx, jnp.int32(-2 ** 31), key)
                ksel = jnp.where(rid == j, mx, ksel)
                am = jnp.clip(S - (mx[0, 0] & 0xFFFF), 0, S - 1)
                idxs.append(am)
                w = xn_ref[pl.ds(lax.shift_right_logical(am, 1), 1), :]
                sh = ((am & 1) * 16).astype(u32)
                rows.append(lax.shift_left(lax.shift_right_logical(w, sh), u32(16)))
            xs = pltpu.bitcast(jnp.concatenate(rows, axis=0), f32)
            ksel = ksel & jnp.int32(-65536)
            rsel = pltpu.bitcast(
                jnp.broadcast_to(jnp.where(ksel < 0, ksel ^ 0x7FFF0000, ksel), (C, 128)), f32)[:, 0:1]
            md.update(xs=xs, xsb=xs.astype(bf16), idxs=idxs, rsel=rsel)

        def mod_gate_up():
            a, u = [jnp.dot(md['xsb'], jnp.concatenate([_upk(wt_ref[mt * NF + t]) for t in range(NF)], axis=1),
                            preferred_element_type=f32) for mt in (0, 1)]
            col = lax.broadcasted_iota(jnp.int32, a.shape, 1)
            dup = jnp.logical_and(col >= (NF - 1) * 128, col < (NF - 1) * 128 + (NF * 128 - F))
            md['hh'] = jnp.where(dup, 0.0, a * _sigmoid(a) * u).astype(bf16)

        def mod_down():
            n0 = (NF - 1) * 128
            y = (jnp.dot(md['hh'][:, :n0], wd_ref[0:n0, :], preferred_element_type=f32)
                 + jnp.dot(md['hh'][:, n0:], wd_ref[F - 128:F, :], preferred_element_type=f32))
            zz = md['xs'] + y * _sigmoid(md['rsel'])
            gb = lax.shift_right_logical(pltpu.bitcast(_rb(_silu(_rb(zz))), u32), u32(16))
            for j, idx in enumerate(md['idxs']):
                row = pl.ds(lax.shift_right_logical(idx, 1), 1)
                sh = ((idx & 1) * 16).astype(u32)
                keep = lax.shift_left(u32(0xFFFF), u32(16) - sh)
                g_ref[row, :] = (g_ref[row, :] & keep) | lax.shift_left(gb[j:j + 1, :], sh)

        def wtr():
            t = h - 1
            real = jnp.logical_and(t >= 0, t < 2 * NF)
            mt = (t >= NF).astype(jnp.int32)
            src = jnp.where(real, mt * F + jnp.minimum((t - mt * NF) * 128, F - 128), 2 * F)
            blk = wgu_ref[pl.ds(pl.multiple_of(src, 64), 128), :]
            wt_ref[jnp.where(real, t, 2 * NF)] = _pk(blk.T)

        def gate_router(k):
            if pre:
                rg = (H - 1) * (GR // 8) + 2 * k
                rows = pl.ds(rg * 4, 8)
            else:
                rg = h * (GR // 8) + 2 * k
                rows = pl.ds(pl.multiple_of(rg * 4, 8), 8)
            xn = _upk(xn_ref[rows, :]).astype(f32)
            g_ref[rows, :] = _pk(_silu(xn).astype(bf16))
            xw = xn * wrf_ref[...]
            rr = [jnp.sum(xw[kk * 8:kk * 8 + 8], axis=-1, keepdims=True) for kk in (0, 1)]
            for v in range(S // 1024):
                r = r_ref[v * 8:v * 8 + 8, :]
                for kk in (0, 1):
                    r = jnp.where(lane == rg + (kk - v * 128), rr[kk], r)
                r_ref[v * 8:v * 8 + 8, :] = r

        lnq = []
        if pre:
            x_cp(0).start()
            f_cp(3).start()
            wq_cp(0).start()
            x_cp(1).start()
            for c in range(5):
                acc_refs[c][...] = jnp.zeros((G, D), f32)
            x_cp(0).wait()
            f_cp(3).wait()
            k_cp(0).start()
            wrf_ref[...] = jnp.broadcast_to(wr_ref[...].astype(f32).reshape(1, D), (16, D))
            r_ref[...] = jnp.zeros(r_ref.shape, f32)
            wgu_ref[2 * F:, :] = jnp.zeros((128, D), bf16)
            ln_group(0)
            for c in range(5, NG):
                acc_refs[c][...] = jnp.zeros((G, D), f32)
            v_cp(0).start()
            x_cp(2).start()
            wo_cp(0).start()
            wq_cp(0).wait()
            x_cp(1).wait()
            wqw_ref[...] = _pk(wqbuf[0:D, :])
            qproj(0)
            ln_group(1)
            x_cp(3).start()
            k_cp(0).wait()
            for j in range(NK):
                kcopy(j)
            lnq = list(range(2 * LNSUB, NG * LNSUB))
            lo, hi = -AHEAD, B
        elif post:
            f_cp(2).wait()
            lo, hi = B, W
        else:
            for cp in (k_cp, v_cp, wq_cp, wo_cp):
                cp(h + 1).wait()

            @pl.when(h == 1)
            def _():
                f_cp(0).wait()
                f_cp(1).wait()
            lo, hi = B, B + W

        if not pre:
            for i, c in enumerate(LIVE_Q):
                qts[c] = _upk(q_c[i])
            for i, c in enumerate(LIVE_MX):
                maccs[c] = m_c[i]
            for i, c in enumerate(LIVE_M):
                ms[c] = m_c[len(LIVE_MX) + i]
            for i, c in enumerate(LIVE_O):
                laccs[c] = l_c[i]
            for i, c in enumerate(LIVE_O):
                oaccs[c] = o_c[i]

        t_prep = lambda c: max(B, (c + 1) * NK + 0.3) if post and p_prep(c) >= B else p_prep(c)
        t_op = lambda c: max(t_prep(c) + 1, B + 6.5 + c) if post else p_oproj(c)
        t_qp = lambda c: (min(max(p_qproj(c), W6 + 0.75), p_qk(c, 0) - 0.25) if pre and c >= 3 else
                          -AHEAD + 0.5 if pre and c == 1 else p_qproj(c))
        t_qk = lambda c, j: max(p_qk(c, j) - 1, W5 - 0.1 + 0.01 * j) if pre and c == 1 else p_qk(c, j)
        lntimes = [t + 0.4 for t in range(W5, W)]

        def ev_qk(c, j):
            qk(c, j)
            if c == NG - 1 and not post:
                kcopy(j)
                if j == NK - 1:
                    refill(k_cp, kbuf)

        def ev_pv(c, j):
            pv(c, j)
            if c == NG - 1 and not post:
                vtr(j)
                if j == NK - 1:
                    refill(v_cp, vbuf)

        def ev_op(c):
            oproj(c)
            if c == NG - 1:
                wow_ref[...] = _pk(wobuf[0:DH, :])
                refill(wo_cp, wobuf)

        def ev_qp(c):
            if c == NG:
                wqw_ref[...] = _pk(wqbuf[0:D, :])
                refill(wq_cp, wqbuf)
            assert not pre or c in lndone, c
            qproj(c)

        def ev_w5():
            v_cp(0).wait()
            x_cp(2).wait()
            wo_cp(0).wait()
            for j in range(NK):
                vtr(j)
            wow_ref[...] = _pk(wobuf[0:DH, :])

        def ev_w6():
            for cp in (k_cp, v_cp, wq_cp, wo_cp):
                cp(1).start()
            x_cp(3).wait()
            for i in range(3):
                f_cp(i).start()

        def ev_ln(pos):
            avail = [t for t in lnq if t < 3 * LNSUB or pos >= W6]
            left = lambda c: max(len([1 for tt in lntimes if pos <= tt < min(t_qp(c), B)]), 1)
            cnt = 1
            for n_, t in enumerate(avail):
                cnt = max(cnt, -(-(n_ + 4) // left(t // LNSUB)))
            for p, sg in lnstage.items():
                cnt = max(cnt, -(-(3 - sg) // left(p // LNSUB)))
            for _ in range(cnt):
                if avail or lnstage:
                    t = avail.pop(0) if avail else None
                    if t is not None:
                        lnq.remove(t)
                    tick(t)

        ev = []
        for c in range(NG if post or pre else 2 * NG + 2):
            for j in range(NK):
                ev.append((t_qk(c, j), ev_qk, (c, j)))
                ev.append((p_pv(c, j), ev_pv, (c, j)))
            if not (post and c == NG - 1):
                ev.append((t_op(c), ev_op, (c,)))
                ev.append((t_prep(c), oprep, (c,)))
            if c >= 1:
                ev.append((t_qp(c), ev_qp, (c,)))
        if pre:
            ev += [(W5 - 0.01, ev_w5, ()), (W6 - 0.01, ev_w6, ())]
            ev += [(t, ev_ln, (t,)) for t in lntimes]
            ev += [(B - 0.001, gate_router, (k,)) for k in range(GR // 16)]
        elif post:
            ev += [(B, mod_select, ()), (B + 4.4, mod_gate_up, ()), (B + 5.45, mod_down, ())]
        else:
            ev += [(20.3 + 4 * k, gate_router, (k,)) for k in range(GR // 16)]
            ev.append((16.1, wtr, ()))
        for _, f, a in sorted([e for e in ev if lo <= e[0] < hi], key=lambda e: e[0]):
            f(*a)

        if post:
            oprep(NG - 1)
            oproj(NG - 1, LASTSUB)
            for c in range(NG - 1):
                o_cp(c).wait()
            for i in range(LASTSUB):
                o_cp(NG - 1, i, LASTSUB).wait()
            return
        assert not lnq and not lnstage
        sh = 0 if pre else NG
        for i, c in enumerate(LIVE_Q):
            q_c[i] = _pk(qs[c + sh].T)
        for i, c in enumerate(LIVE_MX):
            m_c[i] = maccs[c + sh]
        for i, c in enumerate(LIVE_M):
            m_c[len(LIVE_MX) + i] = ms[c + sh]
        for i, c in enumerate(LIVE_O):
            l_c[i] = laccs[c + sh]
        for i, c in enumerate(LIVE_O):
            o_c[i] = oaccs[c + sh]

    zero = zero_ref[0]
    segment(0, 'pre', zero)

    def mid(h, carry):
        segment(h, 'mid', jnp.minimum(h, 0))
        return carry

    lax.fori_loop(0, H - 1, mid, 0)
    segment(H - 1, 'post', zero)


@jax.jit
def pallas_recurrent_scan__mha_block_cached__moe_arch_mod__prompt_kernel(
    A_x: jax.Array,
    A_k_cache: jax.Array,
    A_v_cache: jax.Array,
    A_wq: jax.Array,
    A_wo: jax.Array,
    B_x: jax.Array,
    B_w_r: jax.Array,
    B_w_gate: jax.Array,
    B_w_up: jax.Array,
    B_w_down: jax.Array,
):
    del B_x
    hbm = pl.BlockSpec(memory_space=pl.ANY)
    V = pltpu.VMEM
    dma = pltpu.SemaphoreType.DMA
    out = pl.pallas_call(
        _kernel,
        in_specs=[pl.BlockSpec(memory_space=pltpu.SMEM)] + [hbm] * 9,
        out_specs=hbm,
        out_shape=jax.ShapeDtypeStruct((S, D), bf16),
        scratch_shapes=[
            V((D,), bf16), V((16, D), f32), V((S, D), bf16),
            V((S + 16, DH), bf16), V((S + 16, DH), bf16), V((D + 16, DH), bf16), V((DH + 16, D), bf16),
            V((2 * F + 128, D), bf16), V((2 * NF + 1, D // 2, 128), u32), V((F, D), bf16),
            V((S // 2, D), u32), V((S // 2, D), u32), V((S // 128, 128), f32),
            V((S // 2, DH), u32), V((DH // 2, S), u32), V((D // 2, DH), u32), V((DH // 2, D), u32),
            V((len(LIVE_MX) + len(LIVE_M), 8, G), f32), V((len(LIVE_O), 8, G), f32),
            V((len(LIVE_O), DH, G), f32), V((len(LIVE_Q), DH // 2, G), u32),
            dma((len(XSPLIT),)), dma((4,)), dma((4,)), dma((NG - 1 + LASTSUB,)),
        ] + [V((S, G), f32)] * NSBUF + [V((G // 2, DH), u32)] * NG + [V((G + 16, D), bf16)] * NG
        + [V((G, D), f32)] * NG,
        compiler_params=pltpu.CompilerParams(
            vmem_limit_bytes=100 * 1024 * 1024,
            disable_semaphore_checks=True,
            disable_bounds_checks=True,
        ),
    )(jnp.zeros((1,), jnp.int32), A_x.reshape(S, D), A_k_cache.reshape(H, S, DH), A_v_cache.reshape(H, S, DH),
      A_wq, A_wo, B_w_r, B_w_gate.T, B_w_up.T, B_w_down)
    return out.reshape(1, S, D)
```

```python
import jax
import jax.numpy as jnp
from jax import lax
import jax.experimental.pallas as pl
import jax.experimental.pallas.tpu as pltpu

S, D, H, DH, F, C = 2048, 640, 32, 128, 1728, 8
LOG2E = 1.4426950408889634
NT = (((1,), (1,)), ((), ()))
f32 = jnp.float32
bf16 = jnp.bfloat16
u32 = jnp.uint32

G = 256
KC = 512
NG = S // G
NK = S // KC
W = NG * NK
AHEAD = NK + 1
B = 13
NSBUF = 4
LAG, TAIL_LAG = 2, 4
LNSUB = 4
LR = G // LNSUB
GR = S // H
NF = -(-F // 128)
XSPLIT = (1, 1, 1, NG - 3)
XOFF = tuple(sum(XSPLIT[:i]) for i in range(len(XSPLIT)))
W5, W6 = -1, 5
LASTSUB = 8
TAIL = 3

p_qproj = lambda c: (c - 2) * NK + 1.75
p_qk = lambda c, j: c * NK + j - AHEAD
p_pv = lambda c, j: c * NK + j + 0.25
p_prep = lambda c: (c + 1) * NK + 2.6
p_oproj = lambda c: (c + 1) * NK + 10.5
_rng = range(-2, 2 * NG + 2)
LIVE_Q = [c for c in _rng if p_qproj(c) < B <= p_qk(c, NK - 1)]
LIVE_MX = [c for c in _rng if p_qk(c, 0) < B <= p_pv(c, 0)]
LIVE_M = [c for c in _rng if p_pv(c, 0) < B <= p_pv(c, NK - 1)]
LIVE_O = [c for c in _rng if p_pv(c, 0) < B <= p_prep(c)]
assert p_oproj(0) >= B


def _rb(a):
    return a.astype(bf16).astype(f32)


def _gate(m, tok):
    return jnp.maximum(m, jnp.minimum(m, tok))


def _sigmoid(x):
    return 0.5 * jnp.tanh(0.5 * x) + 0.5


def _silu(x):
    hx = x * 0.5
    return hx * jnp.tanh(hx) + hx


def _pk(a):
    return pltpu.bitcast(a, u32)


def _upk(a):
    return pltpu.bitcast(a, bf16)


def _kernel(zero_ref, x_hbm, k_hbm, v_hbm, wq_hbm, wo_hbm, wr_hbm, wg_hbm, wu_hbm, wd_hbm, o_hbm,
            wr_ref, wrf_ref, x_ref, kbuf, vbuf, wqbuf, wobuf, wgu_ref, wt_ref, wd_ref,
            xn_ref, g_ref, r_ref, kw_ref, vt_ref, wqw_ref, wow_ref,
            m_c, l_c, o_c, q_c,
            xsem, hsem, fsem, osem, *rest):
    s_refs, rest = rest[:NSBUF], rest[NSBUF:]
    o_refs, ob_refs, acc_refs = rest[:NG], rest[NG:2 * NG], rest[2 * NG:]

    def x_cp(i):
        rows = pl.ds(XOFF[i] * G, XSPLIT[i] * G)
        return pltpu.make_async_copy(x_hbm.at[rows, :], x_ref.at[rows, :], xsem.at[i])

    def k_cp(h):
        return pltpu.make_async_copy(k_hbm.at[h], kbuf.at[0:S, :], hsem.at[0])

    def v_cp(h):
        return pltpu.make_async_copy(v_hbm.at[h], vbuf.at[0:S, :], hsem.at[1])

    def wq_cp(h):
        col = h * DH if isinstance(h, int) else pl.multiple_of(h * DH, DH)
        return pltpu.make_async_copy(wq_hbm.at[:, pl.ds(col, DH)], wqbuf.at[0:D, :], hsem.at[2])

    def wo_cp(h):
        row = h * DH if isinstance(h, int) else pl.multiple_of(h * DH, DH)
        return pltpu.make_async_copy(wo_hbm.at[pl.ds(row, DH), :], wobuf.at[0:DH, :], hsem.at[3])

    def f_cp(i):
        src = (wg_hbm, wu_hbm, wd_hbm, wr_hbm)[i]
        dst = (wgu_ref.at[0:F, :], wgu_ref.at[F:2 * F, :], wd_ref, wr_ref)[i]
        return pltpu.make_async_copy(src, dst, fsem.at[i])

    def o_cp(c, i=0, nsub=1):
        n = G // nsub
        return pltpu.make_async_copy(ob_refs[c].at[i * n:(i + 1) * n, :], o_hbm.at[pl.ds(c * G + i * n, n), :],
                                     osem.at[c + i])

    def segment(h, mode, zero):
        pre, post = mode == 'pre', mode == 'post'
        qs, qts, maccs, ms, laccs, oaccs = {}, {}, {}, {}, {}, {}
        hist = {}
        extra = []

        def pin(ref, lagn):
            spare = pl.ds(pl.multiple_of(zero + (ref.shape[0] - 16), 16), 16)
            ref[spare, 0:128] = jnp.zeros((16, 128), bf16)
            t = pltpu.bitcast(ref[spare, 0:128], f32)
            extra.append((len(hist) + lagn, jnp.concatenate([t] * (G // 128), axis=1)))

        def refill(cp, ref):
            @pl.when(h + 2 < H)
            def _():
                cp(h + 2).start()
            pin(ref, 1)

        lane = lax.broadcasted_iota(jnp.int32, (8, 128), 1)

        lnst, lnstage, lndone = {}, {}, set()

        def ln_a(t):
            xs = []
            for r in range(t * LR, (t + 1) * LR, 16):
                x16 = x_ref[r:r + 16, :].astype(f32)
                xs += [x16[:8], x16[8:]]
            lnst[t] = dict(xs=xs, means=[jnp.sum(x, axis=-1, keepdims=True) * (1.0 / D) for x in xs])

        def ln_b(t):
            st = lnst[t]
            ssq = jnp.zeros((8, 128), f32)
            dm = jnp.zeros((8, 128), f32)
            ds = []
            for k, (x, mean) in enumerate(zip(st['xs'], st['means'])):
                mk = _rb(mean)
                d = x - mk
                ds.append(d)
                ssq = jnp.where(lane == k, jnp.sum(d * d, axis=-1, keepdims=True), ssq)
                dm = jnp.where(lane == k, mean - mk, dm)
            st['d'] = [jnp.concatenate(ds[k:k + 2], axis=0).astype(bf16) for k in range(0, LR // 8, 2)]
            var = jnp.maximum(ssq * (1.0 / D) - dm * dm, 0.0)
            st['inv'] = 1.0 / _rb(jnp.sqrt(_rb(_rb(var) + _rb(f32(1e-5)))))

        def ln_b2(t):
            st = lnst[t]
            st['invs'] = [jnp.sum(jnp.where(lane == k, st['inv'], 0.0), axis=-1, keepdims=True)
                          for k in range(LR // 8)]

        def ln_c(t):
            st = lnst.pop(t)
            for k in range(0, LR // 8, 2):
                d = st['d'][k // 2].astype(f32)
                xn = jnp.concatenate([d[:8] * st['invs'][k], d[8:] * st['invs'][k + 1]], axis=0)
                r = t * LR + k * 8
                xn_ref[r // 2:r // 2 + 8, :] = _pk(xn.astype(bf16))
            if (t + 1) % LNSUB == 0:
                lndone.add(t // LNSUB)

        def tick(t):
            for p in sorted(lnstage):
                (ln_b, ln_b2, ln_c)[lnstage[p]](p)
                lnstage[p] += 1
                if lnstage[p] == 3:
                    del lnstage[p]
            if t is not None:
                ln_a(t)
                lnstage[t] = 0

        def ln_group(c):
            for t in range(c * LNSUB, (c + 1) * LNSUB):
                tick(t)
            while lnstage:
                tick(None)

        def qproj(c):
            r0 = (c % NG) * (G // 2)
            q = jnp.dot(_upk(xn_ref[r0:r0 + G // 2, :]), _upk(wqw_ref[...]), preferred_element_type=f32)
            qs[c] = (q * (DH ** -0.5 * LOG2E)).astype(bf16)

        def qk(c, j):
            kk = _upk(kw_ref[j * KC // 2:(j + 1) * KC // 2, :])
            if c in qts:
                st = jnp.dot(kk, qts[c], preferred_element_type=f32)
            else:
                st = lax.dot_general(kk, qs[c], NT, preferred_element_type=f32)
            off = pl.multiple_of(zero + j * KC, KC)
            s_refs[c % NSBUF][pl.ds(off, KC), :] = st
            mm = jnp.max(st.reshape(KC // 8, 8, G), axis=0)
            maccs[c] = mm if j == 0 else jnp.maximum(maccs[c], mm)

        def kcopy(j):
            kw_ref[j * KC // 2:(j + 1) * KC // 2, :] = _pk(kbuf[j * KC:(j + 1) * KC, :])

        def vtr(j):
            vt_ref[:, j * KC:(j + 1) * KC] = _pk(vbuf[j * KC:(j + 1) * KC, :].T)

        def pv(c, j):
            if j == 0:
                ms[c] = jnp.broadcast_to(jnp.max(maccs[c], axis=0, keepdims=True), (8, G))
            m = ms[c]
            n = c * NK + j
            for tok in hist.get(n - (TAIL_LAG if post and n > W - AHEAD else LAG), ()):
                m = _gate(m, tok)
            for e in [e for e in extra if e[0] <= len(hist)]:
                m = _gate(m, e[1])
            extra[:] = [e for e in extra if e[0] > len(hist)]
            vt = _upk(vt_ref[:, j * KC:(j + 1) * KC])
            p = jnp.exp2(s_refs[c % NSBUF][j * KC:(j + 1) * KC, :].reshape(KC // 8, 8, G) - m[None])
            ll = jnp.sum(p, axis=0)
            laccs[c] = ll if j == 0 else laccs[c] + ll
            oo = jnp.dot(vt, p.reshape(KC, G).astype(bf16), preferred_element_type=f32)
            oaccs[c] = oo if j == 0 else oaccs[c] + oo
            hist[n] = [laccs[c], oaccs[c][DH - 8:, :]]

        def oprep(c):
            l = jnp.sum(laccs[c], axis=0, keepdims=True)
            o_refs[c % NG][...] = _pk((oaccs[c] * (1.0 / l)).T.astype(bf16))

        def oproj(c, nsub=1, pieces=None):
            n = G // nsub
            for i in (range(nsub) if pieces is None else pieces):
                y = jnp.dot(_upk(o_refs[c % NG][i * n // 2:(i + 1) * n // 2, :]), _upk(wow_ref[...]),
                            preferred_element_type=f32)
                if not post:
                    acc_refs[c % NG][i * n:(i + 1) * n, :] += y
                else:
                    for r in range(i * n, (i + 1) * n, 16):
                        g = _upk(g_ref[(c * G + r) // 2:(c * G + r) // 2 + 8, :]).astype(f32)
                        sv = acc_refs[c][r:r + 16, :] + y[r - i * n:r - i * n + 16]
                        ob_refs[c][r:r + 16, :] = (x_ref[c * G + r:c * G + r + 16, :].astype(f32) + sv * g).astype(bf16)
                    o_cp(c, i, nsub).start()
            if post and nsub == 1:
                pin(ob_refs[c], 2)

        def tail():
            c = NG - 1
            for t in range(G // 128):
                cols = slice(t * 128, (t + 1) * 128)
                lacc, oacc = laccs[c][:, cols], oaccs[c][:, cols]
                for j in range(NK - TAIL, NK):
                    st = s_refs[c % NSBUF][j * KC:(j + 1) * KC, cols]
                    p = jnp.exp2(st.reshape(KC // 8, 8, 128) - ms[c][:, cols][None])
                    lacc = lacc + jnp.sum(p, axis=0)
                    oacc = oacc + jnp.dot(_upk(vt_ref[:, j * KC:(j + 1) * KC]), p.reshape(KC, 128).astype(bf16),
                                          preferred_element_type=f32)
                if t == 1:
                    oproj(c, LASTSUB, range(LASTSUB // 2))
                l = jnp.sum(lacc, axis=0, keepdims=True)
                o_refs[c][t * 64:(t + 1) * 64, :] = _pk((oacc * (1.0 / l)).T.astype(bf16))
            oproj(c, LASTSUB, range(LASTSUB // 2, LASTSUB))

        md = {}

        def mod_select():
            r = _rb(r_ref[...]) + 0.0
            i0 = lax.broadcasted_iota(jnp.int32, r.shape, 0)
            ids = ((i0 >> 3) * 128 + lax.broadcasted_iota(jnp.int32, r.shape, 1)) * 8 + (i0 & 7)
            bits = pltpu.bitcast(r, jnp.int32)
            hi = jnp.where(bits < 0, bits ^ 0x7FFF0000, bits)
            hi = jnp.where(r != r, jnp.int32(-2 ** 31), hi)
            key = hi | (S - ids)
            rid = lax.broadcasted_iota(jnp.int32, (C, 1), 0)
            ksel = jnp.zeros((C, 1), jnp.int32)
            idxs, rows = [], []
            for j in range(C):
                mx = jnp.max(key, keepdims=True)
                key = jnp.where(key == mx, jnp.int32(-2 ** 31), key)
                ksel = jnp.where(rid == j, mx, ksel)
                am = jnp.clip(S - (mx[0, 0] & 0xFFFF), 0, S - 1)
                idxs.append(am)
                w = xn_ref[pl.ds(lax.shift_right_logical(am, 1), 1), :]
                sh = ((am & 1) * 16).astype(u32)
                rows.append(lax.shift_left(lax.shift_right_logical(w, sh), u32(16)))
            xs = pltpu.bitcast(jnp.concatenate(rows, axis=0), f32)
            ksel = ksel & jnp.int32(-65536)
            rsel = pltpu.bitcast(
                jnp.broadcast_to(jnp.where(ksel < 0, ksel ^ 0x7FFF0000, ksel), (C, 128)), f32)[:, 0:1]
            md.update(xs=xs, xsb=xs.astype(bf16), idxs=idxs, rsel=rsel)

        def mod_gate_up():
            a, u = [jnp.dot(md['xsb'], jnp.concatenate([_upk(wt_ref[mt * NF + t]) for t in range(NF)], axis=1),
                            preferred_element_type=f32) for mt in (0, 1)]
            col = lax.broadcasted_iota(jnp.int32, a.shape, 1)
            dup = jnp.logical_and(col >= (NF - 1) * 128, col < (NF - 1) * 128 + (NF * 128 - F))
            md['hh'] = jnp.where(dup, 0.0, a * _sigmoid(a) * u).astype(bf16)

        def mod_down():
            n0 = (NF - 1) * 128
            y = (jnp.dot(md['hh'][:, :n0], wd_ref[0:n0, :], preferred_element_type=f32)
                 + jnp.dot(md['hh'][:, n0:], wd_ref[F - 128:F, :], preferred_element_type=f32))
            zz = md['xs'] + y * _sigmoid(md['rsel'])
            gb = lax.shift_right_logical(pltpu.bitcast(_rb(_silu(_rb(zz))), u32), u32(16))
            for j, idx in enumerate(md['idxs']):
                row = pl.ds(lax.shift_right_logical(idx, 1), 1)
                sh = ((idx & 1) * 16).astype(u32)
                keep = lax.shift_left(u32(0xFFFF), u32(16) - sh)
                g_ref[row, :] = (g_ref[row, :] & keep) | lax.shift_left(gb[j:j + 1, :], sh)

        def wtr():
            t = h - 1
            real = jnp.logical_and(t >= 0, t < 2 * NF)
            mt = (t >= NF).astype(jnp.int32)
            src = jnp.where(real, mt * F + jnp.minimum((t - mt * NF) * 128, F - 128), 2 * F)
            blk = wgu_ref[pl.ds(pl.multiple_of(src, 64), 128), :]
            wt_ref[jnp.where(real, t, 2 * NF)] = _pk(blk.T)

        def gate_router(k):
            if pre:
                rg = (H - 1) * (GR // 8) + 2 * k
                rows = pl.ds(rg * 4, 8)
            else:
                rg = h * (GR // 8) + 2 * k
                rows = pl.ds(pl.multiple_of(rg * 4, 8), 8)
            xn = _upk(xn_ref[rows, :]).astype(f32)
            g_ref[rows, :] = _pk(_silu(xn).astype(bf16))
            xw = xn * wrf_ref[...]
            rr = [jnp.sum(xw[kk * 8:kk * 8 + 8], axis=-1, keepdims=True) for kk in (0, 1)]
            for v in range(S // 1024):
                r = r_ref[v * 8:v * 8 + 8, :]
                for kk in (0, 1):
                    r = jnp.where(lane == rg + (kk - v * 128), rr[kk], r)
                r_ref[v * 8:v * 8 + 8, :] = r

        lnq = []
        if pre:
            x_cp(0).start()
            f_cp(3).start()
            wq_cp(0).start()
            x_cp(1).start()
            for c in range(5):
                acc_refs[c][...] = jnp.zeros((G, D), f32)
            x_cp(0).wait()
            f_cp(3).wait()
            k_cp(0).start()
            wrf_ref[...] = jnp.broadcast_to(wr_ref[...].astype(f32).reshape(1, D), (16, D))
            r_ref[...] = jnp.zeros(r_ref.shape, f32)
            wgu_ref[2 * F:, :] = jnp.zeros((128, D), bf16)
            ln_group(0)
            for c in range(5, NG):
                acc_refs[c][...] = jnp.zeros((G, D), f32)
            v_cp(0).start()
            x_cp(2).start()
            wo_cp(0).start()
            wq_cp(0).wait()
            x_cp(1).wait()
            wqw_ref[...] = _pk(wqbuf[0:D, :])
            qproj(0)
            ln_group(1)
            x_cp(3).start()
            k_cp(0).wait()
            for j in range(NK):
                kcopy(j)
            lnq = list(range(2 * LNSUB, NG * LNSUB))
            lo, hi = -AHEAD, B
        elif post:
            f_cp(2).wait()
            lo, hi = B, W
        else:
            for cp in (k_cp, v_cp, wq_cp, wo_cp):
                cp(h + 1).wait()

            @pl.when(h == 1)
            def _():
                f_cp(0).wait()
                f_cp(1).wait()
            lo, hi = B, B + W

        if not pre:
            for i, c in enumerate(LIVE_Q):
                qts[c] = _upk(q_c[i])
            for i, c in enumerate(LIVE_MX):
                maccs[c] = m_c[i]
            for i, c in enumerate(LIVE_M):
                ms[c] = m_c[len(LIVE_MX) + i]
            for i, c in enumerate(LIVE_O):
                laccs[c] = l_c[i]
            for i, c in enumerate(LIVE_O):
                oaccs[c] = o_c[i]

        t_prep = lambda c: max(B, (c + 1) * NK + 0.3) if post and p_prep(c) >= B else p_prep(c)
        t_op = lambda c: max(t_prep(c) + 1, B + 6.5 + c) if post else p_oproj(c)
        t_qp = lambda c: (min(max(p_qproj(c), W6 + 0.75), p_qk(c, 0) - 0.25) if pre and c >= 3 else
                          -AHEAD + 0.5 if pre and c == 1 else p_qproj(c))
        t_qk = lambda c, j: max(p_qk(c, j) - 1, W5 - 0.1 + 0.01 * j) if pre and c == 1 else p_qk(c, j)
        lntimes = [t + 0.4 for t in range(W5, W)]

        def ev_qk(c, j):
            qk(c, j)
            if c == NG - 1 and not post:
                kcopy(j)
                if j == NK - 1:
                    refill(k_cp, kbuf)

        def ev_pv(c, j):
            pv(c, j)
            if c == NG - 1 and not post:
                vtr(j)
                if j == NK - 1:
                    refill(v_cp, vbuf)

        def ev_op(c):
            oproj(c)
            if c == NG - 1:
                wow_ref[...] = _pk(wobuf[0:DH, :])
                refill(wo_cp, wobuf)

        def ev_qp(c):
            if c == NG:
                wqw_ref[...] = _pk(wqbuf[0:D, :])
                refill(wq_cp, wqbuf)
            assert not pre or c in lndone, c
            qproj(c)

        def ev_w5():
            v_cp(0).wait()
            x_cp(2).wait()
            wo_cp(0).wait()
            for j in range(NK):
                vtr(j)
            wow_ref[...] = _pk(wobuf[0:DH, :])

        def ev_w6():
            for cp in (k_cp, v_cp, wq_cp, wo_cp):
                cp(1).start()
            x_cp(3).wait()
            for i in range(3):
                f_cp(i).start()

        def ev_ln(pos):
            avail = [t for t in lnq if t < 3 * LNSUB or pos >= W6]
            left = lambda c: max(len([1 for tt in lntimes if pos <= tt < min(t_qp(c), B)]), 1)
            cnt = 1
            for n_, t in enumerate(avail):
                cnt = max(cnt, -(-(n_ + 4) // left(t // LNSUB)))
            for p, sg in lnstage.items():
                cnt = max(cnt, -(-(3 - sg) // left(p // LNSUB)))
            for _ in range(cnt):
                if avail or lnstage:
                    t = avail.pop(0) if avail else None
                    if t is not None:
                        lnq.remove(t)
                    tick(t)

        ev = []
        for c in range(NG if post or pre else 2 * NG + 2):
            for j in range(NK):
                ev.append((t_qk(c, j), ev_qk, (c, j)))
                if not (post and c == NG - 1 and j >= NK - TAIL):
                    ev.append((p_pv(c, j), ev_pv, (c, j)))
            if not (post and c == NG - 1):
                ev.append((t_op(c), ev_op, (c,)))
                ev.append((t_prep(c), oprep, (c,)))
            if c >= 1:
                ev.append((t_qp(c), ev_qp, (c,)))
        if pre:
            ev += [(W5 - 0.01, ev_w5, ()), (W6 - 0.01, ev_w6, ())]
            ev += [(t, ev_ln, (t,)) for t in lntimes]
            ev += [(B - 0.001, gate_router, (k,)) for k in range(GR // 16)]
        elif post:
            ev += [(B, mod_select, ()), (B + 4.4, mod_gate_up, ()), (B + 5.45, mod_down, ())]
        else:
            ev += [(20.3 + 4 * k, gate_router, (k,)) for k in range(GR // 16)]
            ev.append((16.1, wtr, ()))
        for _, f, a in sorted([e for e in ev if lo <= e[0] < hi], key=lambda e: e[0]):
            f(*a)

        if post:
            tail()
            for c in range(NG - 1):
                o_cp(c).wait()
            for i in range(LASTSUB):
                o_cp(NG - 1, i, LASTSUB).wait()
            return
        assert not lnq and not lnstage
        sh = 0 if pre else NG
        for i, c in enumerate(LIVE_Q):
            q_c[i] = _pk(qs[c + sh].T)
        for i, c in enumerate(LIVE_MX):
            m_c[i] = maccs[c + sh]
        for i, c in enumerate(LIVE_M):
            m_c[len(LIVE_MX) + i] = ms[c + sh]
        for i, c in enumerate(LIVE_O):
            l_c[i] = laccs[c + sh]
        for i, c in enumerate(LIVE_O):
            o_c[i] = oaccs[c + sh]

    zero = zero_ref[0]
    segment(0, 'pre', zero)

    def mid(h, carry):
        segment(h, 'mid', jnp.minimum(h, 0))
        return carry

    lax.fori_loop(0, H - 1, mid, 0)
    segment(H - 1, 'post', zero)


@jax.jit
def pallas_recurrent_scan__mha_block_cached__moe_arch_mod__prompt_kernel(
    A_x: jax.Array,
    A_k_cache: jax.Array,
    A_v_cache: jax.Array,
    A_wq: jax.Array,
    A_wo: jax.Array,
    B_x: jax.Array,
    B_w_r: jax.Array,
    B_w_gate: jax.Array,
    B_w_up: jax.Array,
    B_w_down: jax.Array,
):
    del B_x
    hbm = pl.BlockSpec(memory_space=pl.ANY)
    V = pltpu.VMEM
    dma = pltpu.SemaphoreType.DMA
    out = pl.pallas_call(
        _kernel,
        in_specs=[pl.BlockSpec(memory_space=pltpu.SMEM)] + [hbm] * 9,
        out_specs=hbm,
        out_shape=jax.ShapeDtypeStruct((S, D), bf16),
        scratch_shapes=[
            V((D,), bf16), V((16, D), f32), V((S, D), bf16),
            V((S + 16, DH), bf16), V((S + 16, DH), bf16), V((D + 16, DH), bf16), V((DH + 16, D), bf16),
            V((2 * F + 128, D), bf16), V((2 * NF + 1, D // 2, 128), u32), V((F, D), bf16),
            V((S // 2, D), u32), V((S // 2, D), u32), V((S // 128, 128), f32),
            V((S // 2, DH), u32), V((DH // 2, S), u32), V((D // 2, DH), u32), V((DH // 2, D), u32),
            V((len(LIVE_MX) + len(LIVE_M), 8, G), f32), V((len(LIVE_O), 8, G), f32),
            V((len(LIVE_O), DH, G), f32), V((len(LIVE_Q), DH // 2, G), u32),
            dma((len(XSPLIT),)), dma((4,)), dma((4,)), dma((NG - 1 + LASTSUB,)),
        ] + [V((S, G), f32)] * NSBUF + [V((G // 2, DH), u32)] * NG + [V((G + 16, D), bf16)] * NG
        + [V((G, D), f32)] * NG,
        compiler_params=pltpu.CompilerParams(
            vmem_limit_bytes=100 * 1024 * 1024,
            disable_semaphore_checks=True,
            disable_bounds_checks=True,
        ),
    )(jnp.zeros((1,), jnp.int32), A_x.reshape(S, D), A_k_cache.reshape(H, S, DH), A_v_cache.reshape(H, S, DH),
      A_wq, A_wo, B_w_r, B_w_gate.T, B_w_up.T, B_w_down)
    return out.reshape(1, S, D)
```

```python
import jax
import jax.numpy as jnp
from jax import lax
import jax.experimental.pallas as pl
import jax.experimental.pallas.tpu as pltpu

S, D, H, DH, F, C = 2048, 640, 32, 128, 1728, 8
LOG2E = 1.4426950408889634
NT = (((1,), (1,)), ((), ()))
f32 = jnp.float32
bf16 = jnp.bfloat16
u32 = jnp.uint32

G = 256
KC = 512
NG = S // G
NK = S // KC
W = NG * NK
AHEAD = NK + 1
B = 13
NSBUF = 4
LAG = 2
LNSUB = 4
LR = G // LNSUB
GR = S // H
NF = -(-F // 128)
XSPLIT = (1, 1, 1, NG - 3)
XOFF = tuple(sum(XSPLIT[:i]) for i in range(len(XSPLIT)))
W5, W6 = -1, 5
LASTSUB = 8
TAIL = 3

p_qproj = lambda c: (c - 2) * NK + 1.75
p_qk = lambda c, j: c * NK + j - AHEAD
p_pv = lambda c, j: c * NK + j + 0.25
p_prep = lambda c: (c + 1) * NK + 2.6
p_oproj = lambda c: (c + 1) * NK + 10.5
_rng = range(-2, 2 * NG + 2)
LIVE_Q = [c for c in _rng if p_qproj(c) < B <= p_qk(c, NK - 1)]
LIVE_MX = [c for c in _rng if p_qk(c, 0) < B <= p_pv(c, 0)]
LIVE_M = [c for c in _rng if p_pv(c, 0) < B <= p_pv(c, NK - 1)]
LIVE_O = [c for c in _rng if p_pv(c, 0) < B <= p_prep(c)]
assert p_oproj(0) >= B


def _rb(a):
    return a.astype(bf16).astype(f32)


def _gate(m, tok):
    return jnp.maximum(m, jnp.minimum(m, tok))


def _sigmoid(x):
    return 0.5 * jnp.tanh(0.5 * x) + 0.5


def _silu(x):
    hx = x * 0.5
    return hx * jnp.tanh(hx) + hx


def _pk(a):
    return pltpu.bitcast(a, u32)


def _upk(a):
    return pltpu.bitcast(a, bf16)


def _kernel(zero_ref, x_hbm, k_hbm, v_hbm, wq_hbm, wo_hbm, wr_hbm, wg_hbm, wu_hbm, wd_hbm, o_hbm,
            wr_ref, wrf_ref, x_ref, kbuf, vbuf, wqbuf, wobuf, wgu_ref, wt_ref, wd_ref,
            xn_ref, g_ref, r_ref, kw_ref, vt_ref, wqw_ref, wow_ref,
            m_c, l_c, o_c, q_c,
            xsem, hsem, fsem, osem, *rest):
    s_refs, rest = rest[:NSBUF], rest[NSBUF:]
    o_refs, ob_refs, acc_refs = rest[:NG], rest[NG:2 * NG], rest[2 * NG:]

    def x_cp(i):
        rows = pl.ds(XOFF[i] * G, XSPLIT[i] * G)
        return pltpu.make_async_copy(x_hbm.at[rows, :], x_ref.at[rows, :], xsem.at[i])

    def k_cp(h):
        return pltpu.make_async_copy(k_hbm.at[h], kbuf.at[0:S, :], hsem.at[0])

    def v_cp(h):
        return pltpu.make_async_copy(v_hbm.at[h], vbuf.at[0:S, :], hsem.at[1])

    def wq_cp(h):
        col = h * DH if isinstance(h, int) else pl.multiple_of(h * DH, DH)
        return pltpu.make_async_copy(wq_hbm.at[:, pl.ds(col, DH)], wqbuf.at[0:D, :], hsem.at[2])

    def wo_cp(h):
        row = h * DH if isinstance(h, int) else pl.multiple_of(h * DH, DH)
        return pltpu.make_async_copy(wo_hbm.at[pl.ds(row, DH), :], wobuf.at[0:DH, :], hsem.at[3])

    def f_cp(i):
        src = (wg_hbm, wu_hbm, wd_hbm, wr_hbm)[i]
        dst = (wgu_ref.at[0:F, :], wgu_ref.at[F:2 * F, :], wd_ref, wr_ref)[i]
        return pltpu.make_async_copy(src, dst, fsem.at[i])

    def o_cp(c, i=0, nsub=1):
        n = G // nsub
        return pltpu.make_async_copy(ob_refs[c].at[i * n:(i + 1) * n, :], o_hbm.at[pl.ds(c * G + i * n, n), :],
                                     osem.at[c + i])

    def segment(h, mode, zero):
        pre, post = mode == 'pre', mode == 'post'
        qs, qts, maccs, ms, laccs, oaccs = {}, {}, {}, {}, {}, {}
        hist = {}
        extra = []

        def pin(ref, lagn):
            spare = pl.ds(pl.multiple_of(zero + (ref.shape[0] - 16), 16), 16)
            ref[spare, 0:128] = jnp.zeros((16, 128), bf16)
            t = pltpu.bitcast(ref[spare, 0:128], f32)
            extra.append((len(hist) + lagn, jnp.concatenate([t] * (G // 128), axis=1)))

        def refill(cp, ref):
            @pl.when(h + 2 < H)
            def _():
                cp(h + 2).start()
            pin(ref, 1)

        lane = lax.broadcasted_iota(jnp.int32, (8, 128), 1)

        def colsum(p):
            n, nacc = p.shape[0], (64 if pre else 6 if post else 1)
            vs = [jnp.sum(p[i * n // nacc:(i + 1) * n // nacc], axis=0) for i in range(nacc)]
            while len(vs) > 1:
                vs = [vs[i] + vs[i + 1] if i + 1 < len(vs) else vs[i] for i in range(0, len(vs), 2)]
            return vs[0]

        lnst, lnstage, lndone = {}, {}, set()

        def ln_a(t):
            xs = []
            for r in range(t * LR, (t + 1) * LR, 16):
                x16 = x_ref[r:r + 16, :].astype(f32)
                xs += [x16[:8], x16[8:]]
            lnst[t] = dict(xs=xs, means=[jnp.sum(x, axis=-1, keepdims=True) * (1.0 / D) for x in xs])

        def ln_b(t):
            st = lnst[t]
            ssq = jnp.zeros((8, 128), f32)
            dm = jnp.zeros((8, 128), f32)
            ds = []
            for k, (x, mean) in enumerate(zip(st['xs'], st['means'])):
                mk = _rb(mean)
                d = x - mk
                ds.append(d)
                ssq = jnp.where(lane == k, jnp.sum(d * d, axis=-1, keepdims=True), ssq)
                dm = jnp.where(lane == k, mean - mk, dm)
            st['d'] = [jnp.concatenate(ds[k:k + 2], axis=0).astype(bf16) for k in range(0, LR // 8, 2)]
            var = jnp.maximum(ssq * (1.0 / D) - dm * dm, 0.0)
            st['inv'] = 1.0 / _rb(jnp.sqrt(_rb(_rb(var) + _rb(f32(1e-5)))))

        def ln_b2(t):
            st = lnst[t]
            st['invs'] = [jnp.sum(jnp.where(lane == k, st['inv'], 0.0), axis=-1, keepdims=True)
                          for k in range(LR // 8)]

        def ln_c(t):
            st = lnst.pop(t)
            for k in range(0, LR // 8, 2):
                d = st['d'][k // 2].astype(f32)
                xn = jnp.concatenate([d[:8] * st['invs'][k], d[8:] * st['invs'][k + 1]], axis=0)
                r = t * LR + k * 8
                xn_ref[r // 2:r // 2 + 8, :] = _pk(xn.astype(bf16))
            if (t + 1) % LNSUB == 0:
                lndone.add(t // LNSUB)

        def tick(t):
            for p in sorted(lnstage):
                (ln_b, ln_b2, ln_c)[lnstage[p]](p)
                lnstage[p] += 1
                if lnstage[p] == 3:
                    del lnstage[p]
            if t is not None:
                ln_a(t)
                lnstage[t] = 0

        def ln_group(c):
            for t in range(c * LNSUB, (c + 1) * LNSUB):
                tick(t)
            while lnstage:
                tick(None)

        def qproj(c):
            r0 = (c % NG) * (G // 2)
            q = jnp.dot(_upk(xn_ref[r0:r0 + G // 2, :]), _upk(wqw_ref[...]), preferred_element_type=f32)
            qs[c] = (q * (DH ** -0.5 * LOG2E)).astype(bf16)

        def qk(c, j):
            kk = _upk(kw_ref[j * KC // 2:(j + 1) * KC // 2, :])
            if c in qts:
                st = jnp.dot(kk, qts[c], preferred_element_type=f32)
            else:
                st = lax.dot_general(kk, qs[c], NT, preferred_element_type=f32)
            off = pl.multiple_of(zero + j * KC, KC)
            s_refs[c % NSBUF][pl.ds(off, KC), :] = st
            mm = jnp.max(st.reshape(KC // 8, 8, G), axis=0)
            maccs[c] = mm if j == 0 else jnp.maximum(maccs[c], mm)

        def kcopy(j):
            kw_ref[j * KC // 2:(j + 1) * KC // 2, :] = _pk(kbuf[j * KC:(j + 1) * KC, :])

        def vtr(j):
            vt_ref[:, j * KC:(j + 1) * KC] = _pk(vbuf[j * KC:(j + 1) * KC, :].T)

        def pv(c, j):
            if j == 0:
                ms[c] = jnp.broadcast_to(jnp.max(maccs[c], axis=0, keepdims=True), (8, G))
            m = ms[c]
            n = c * NK + j
            for tok in hist.get(n - LAG, ()):
                m = _gate(m, tok)
            for e in [e for e in extra if e[0] <= len(hist)]:
                m = _gate(m, e[1])
            extra[:] = [e for e in extra if e[0] > len(hist)]
            vt = _upk(vt_ref[:, j * KC:(j + 1) * KC])
            p = jnp.exp2(s_refs[c % NSBUF][j * KC:(j + 1) * KC, :].reshape(KC // 8, 8, G) - m[None])
            ll = colsum(p)
            laccs[c] = ll if j == 0 else laccs[c] + ll
            oo = jnp.dot(vt, p.reshape(KC, G).astype(bf16), preferred_element_type=f32)
            oaccs[c] = oo if j == 0 else oaccs[c] + oo
            hist[n] = ([] if pre else [laccs[c]]) + [oaccs[c][DH - 8:, :]]

        def oprep(c):
            l = jnp.sum(laccs[c], axis=0, keepdims=True)
            o_refs[c % NG][...] = _pk((oaccs[c] * (1.0 / l)).T.astype(bf16))

        def oproj(c, nsub=1, pieces=None):
            n = G // nsub
            for i in (range(nsub) if pieces is None else pieces):
                y = jnp.dot(_upk(o_refs[c % NG][i * n // 2:(i + 1) * n // 2, :]), _upk(wow_ref[...]),
                            preferred_element_type=f32)
                if not post:
                    acc_refs[c % NG][i * n:(i + 1) * n, :] += y
                else:
                    for r in range(i * n, (i + 1) * n, 16):
                        g = _upk(g_ref[(c * G + r) // 2:(c * G + r) // 2 + 8, :]).astype(f32)
                        sv = acc_refs[c][r:r + 16, :] + y[r - i * n:r - i * n + 16]
                        ob_refs[c][r:r + 16, :] = (x_ref[c * G + r:c * G + r + 16, :].astype(f32) + sv * g).astype(bf16)
                    o_cp(c, i, nsub).start()
            if post and nsub == 1:
                pin(ob_refs[c], 2)

        def tail():
            c = NG - 1
            for t in range(G // 128):
                cols = slice(t * 128, (t + 1) * 128)
                lacc, oacc = laccs[c][:, cols], oaccs[c][:, cols]
                for j in range(NK - TAIL, NK):
                    st = s_refs[c % NSBUF][j * KC:(j + 1) * KC, cols]
                    p = jnp.exp2(st.reshape(KC // 8, 8, 128) - ms[c][:, cols][None])
                    lacc = lacc + colsum(p)
                    oacc = oacc + jnp.dot(_upk(vt_ref[:, j * KC:(j + 1) * KC]), p.reshape(KC, 128).astype(bf16),
                                          preferred_element_type=f32)
                if t == 1:
                    oproj(c, LASTSUB, range(LASTSUB // 2))
                l = jnp.sum(lacc, axis=0, keepdims=True)
                o_refs[c][t * 64:(t + 1) * 64, :] = _pk((oacc * (1.0 / l)).T.astype(bf16))
            oproj(c, LASTSUB, range(LASTSUB // 2, LASTSUB))

        md = {}

        def mod_select():
            r = _rb(r_ref[...]) + 0.0
            i0 = lax.broadcasted_iota(jnp.int32, r.shape, 0)
            ids = ((i0 >> 3) * 128 + lax.broadcasted_iota(jnp.int32, r.shape, 1)) * 8 + (i0 & 7)
            bits = pltpu.bitcast(r, jnp.int32)
            hi = jnp.where(bits < 0, bits ^ 0x7FFF0000, bits)
            hi = jnp.where(r != r, jnp.int32(-2 ** 31), hi)
            key = hi | (S - ids)
            rid = lax.broadcasted_iota(jnp.int32, (C, 1), 0)
            ksel = jnp.zeros((C, 1), jnp.int32)
            idxs, rows = [], []
            for j in range(C):
                mx = jnp.max(key, keepdims=True)
                key = jnp.where(key == mx, jnp.int32(-2 ** 31), key)
                ksel = jnp.where(rid == j, mx, ksel)
                am = jnp.clip(S - (mx[0, 0] & 0xFFFF), 0, S - 1)
                idxs.append(am)
                w = xn_ref[pl.ds(lax.shift_right_logical(am, 1), 1), :]
                sh = ((am & 1) * 16).astype(u32)
                rows.append(lax.shift_left(lax.shift_right_logical(w, sh), u32(16)))
            xs = pltpu.bitcast(jnp.concatenate(rows, axis=0), f32)
            ksel = ksel & jnp.int32(-65536)
            rsel = pltpu.bitcast(
                jnp.broadcast_to(jnp.where(ksel < 0, ksel ^ 0x7FFF0000, ksel), (C, 128)), f32)[:, 0:1]
            md.update(xs=xs, xsb=xs.astype(bf16), idxs=idxs, rsel=rsel)

        def mod_gate_up():
            a, u = [jnp.dot(md['xsb'], jnp.concatenate([_upk(wt_ref[mt * NF + t]) for t in range(NF)], axis=1),
                            preferred_element_type=f32) for mt in (0, 1)]
            col = lax.broadcasted_iota(jnp.int32, a.shape, 1)
            dup = jnp.logical_and(col >= (NF - 1) * 128, col < (NF - 1) * 128 + (NF * 128 - F))
            md['hh'] = jnp.where(dup, 0.0, a * _sigmoid(a) * u).astype(bf16)

        def mod_down():
            n0 = (NF - 1) * 128
            y = (jnp.dot(md['hh'][:, :n0], wd_ref[0:n0, :], preferred_element_type=f32)
                 + jnp.dot(md['hh'][:, n0:], wd_ref[F - 128:F, :], preferred_element_type=f32))
            zz = md['xs'] + y * _sigmoid(md['rsel'])
            gb = lax.shift_right_logical(pltpu.bitcast(_rb(_silu(_rb(zz))), u32), u32(16))
            for j, idx in enumerate(md['idxs']):
                row = pl.ds(lax.shift_right_logical(idx, 1), 1)
                sh = ((idx & 1) * 16).astype(u32)
                keep = lax.shift_left(u32(0xFFFF), u32(16) - sh)
                g_ref[row, :] = (g_ref[row, :] & keep) | lax.shift_left(gb[j:j + 1, :], sh)

        def wtr():
            t = h - 1
            real = jnp.logical_and(t >= 0, t < 2 * NF)
            mt = (t >= NF).astype(jnp.int32)
            src = jnp.where(real, mt * F + jnp.minimum((t - mt * NF) * 128, F - 128), 2 * F)
            blk = wgu_ref[pl.ds(pl.multiple_of(src, 64), 128), :]
            wt_ref[jnp.where(real, t, 2 * NF)] = _pk(blk.T)

        def gate_router(k):
            if pre:
                rg = (H - 1) * (GR // 8) + 2 * k
                rows = pl.ds(rg * 4, 8)
            else:
                rg = h * (GR // 8) + 2 * k
                rows = pl.ds(pl.multiple_of(rg * 4, 8), 8)
            xn = _upk(xn_ref[rows, :]).astype(f32)
            g_ref[rows, :] = _pk(_silu(xn).astype(bf16))
            xw = xn * wrf_ref[...]
            rr = [jnp.sum(xw[kk * 8:kk * 8 + 8], axis=-1, keepdims=True) for kk in (0, 1)]
            for v in range(S // 1024):
                r = r_ref[v * 8:v * 8 + 8, :]
                for kk in (0, 1):
                    r = jnp.where(lane == rg + (kk - v * 128), rr[kk], r)
                r_ref[v * 8:v * 8 + 8, :] = r

        lnq = []
        if pre:
            x_cp(0).start()
            f_cp(3).start()
            wq_cp(0).start()
            x_cp(1).start()
            for c in range(5):
                acc_refs[c][...] = jnp.zeros((G, D), f32)
            x_cp(0).wait()
            f_cp(3).wait()
            k_cp(0).start()
            wrf_ref[...] = jnp.broadcast_to(wr_ref[...].astype(f32).reshape(1, D), (16, D))
            r_ref[...] = jnp.zeros(r_ref.shape, f32)
            wgu_ref[2 * F:, :] = jnp.zeros((128, D), bf16)
            ln_group(0)
            for c in range(5, NG):
                acc_refs[c][...] = jnp.zeros((G, D), f32)
            v_cp(0).start()
            x_cp(2).start()
            wo_cp(0).start()
            wq_cp(0).wait()
            x_cp(1).wait()
            wqw_ref[...] = _pk(wqbuf[0:D, :])
            qproj(0)
            ln_group(1)
            x_cp(3).start()
            k_cp(0).wait()
            for j in range(NK):
                kcopy(j)
            lnq = list(range(2 * LNSUB, NG * LNSUB))
            lo, hi = -AHEAD, B
        elif post:
            f_cp(2).wait()
            lo, hi = B, W
        else:
            for cp in (k_cp, v_cp, wq_cp, wo_cp):
                cp(h + 1).wait()

            @pl.when(h == 1)
            def _():
                f_cp(0).wait()
                f_cp(1).wait()
            lo, hi = B, B + W

        if not pre:
            for i, c in enumerate(LIVE_Q):
                qts[c] = _upk(q_c[i])
            for i, c in enumerate(LIVE_MX):
                maccs[c] = m_c[i]
            for i, c in enumerate(LIVE_M):
                ms[c] = m_c[len(LIVE_MX) + i]
            for i, c in enumerate(LIVE_O):
                laccs[c] = l_c[i]
            for i, c in enumerate(LIVE_O):
                oaccs[c] = o_c[i]

        t_prep = lambda c: max(B, (c + 1) * NK + 0.3) if post and p_prep(c) >= B else p_prep(c)
        t_op = lambda c: max(t_prep(c) + 0.5, B + 6.5 + c) if post else p_oproj(c)
        t_qp = lambda c: (min(max(p_qproj(c), W6 + 0.75), p_qk(c, 0) - 0.25) if pre and c >= 3 else
                          -AHEAD + 0.5 if pre and c == 1 else p_qproj(c))
        t_qk = lambda c, j: max(p_qk(c, j) - 1, W5 - 0.1 + 0.01 * j) if pre and c == 1 else p_qk(c, j)
        lntimes = [t + 0.4 for t in range(W5, W)]

        def ev_qk(c, j):
            qk(c, j)
            if c == NG - 1 and not post:
                kcopy(j)
                if j == NK - 1:
                    refill(k_cp, kbuf)

        def ev_pv(c, j):
            pv(c, j)
            if c == NG - 1 and not post:
                vtr(j)
                if j == NK - 1:
                    refill(v_cp, vbuf)

        def ev_op(c):
            oproj(c)
            if c == NG - 1:
                wow_ref[...] = _pk(wobuf[0:DH, :])
                refill(wo_cp, wobuf)

        def ev_qp(c):
            if c == NG:
                wqw_ref[...] = _pk(wqbuf[0:D, :])
                refill(wq_cp, wqbuf)
            assert not pre or c in lndone, c
            qproj(c)

        def ev_w5():
            v_cp(0).wait()
            x_cp(2).wait()
            wo_cp(0).wait()
            for j in range(NK):
                vtr(j)
            wow_ref[...] = _pk(wobuf[0:DH, :])

        def ev_w6():
            for cp in (k_cp, v_cp, wq_cp, wo_cp):
                cp(1).start()
            x_cp(3).wait()
            for i in range(3):
                f_cp(i).start()

        def ev_ln(pos):
            avail = [t for t in lnq if t < 3 * LNSUB or pos >= W6]
            left = lambda c: max(len([1 for tt in lntimes if pos <= tt < min(t_qp(c), B)]), 1)
            cnt = 1
            for n_, t in enumerate(avail):
                cnt = max(cnt, -(-(n_ + 4) // left(t // LNSUB)))
            for p, sg in lnstage.items():
                cnt = max(cnt, -(-(3 - sg) // left(p // LNSUB)))
            for _ in range(cnt):
                if avail or lnstage:
                    t = avail.pop(0) if avail else None
                    if t is not None:
                        lnq.remove(t)
                    tick(t)

        ev = []
        for c in range(NG if post or pre else 2 * NG + 2):
            for j in range(NK):
                ev.append((t_qk(c, j), ev_qk, (c, j)))
                if not (post and c == NG - 1 and j >= NK - TAIL):
                    ev.append((p_pv(c, j), ev_pv, (c, j)))
            if not (post and c == NG - 1):
                ev.append((t_op(c), ev_op, (c,)))
                ev.append((t_prep(c), oprep, (c,)))
            if c >= 1:
                ev.append((t_qp(c), ev_qp, (c,)))
        if pre:
            ev += [(W5 - 0.01, ev_w5, ()), (W6 - 0.01, ev_w6, ())]
            ev += [(t, ev_ln, (t,)) for t in lntimes]
            ev += [(B - 0.001, gate_router, (k,)) for k in range(GR // 16)]
        elif post:
            ev += [(B, mod_select, ()), (B + 4.4, mod_gate_up, ()), (B + 5.45, mod_down, ())]
        else:
            ev += [(20.3 + 4 * k, gate_router, (k,)) for k in range(GR // 16)]
            ev.append((16.1, wtr, ()))
        for _, f, a in sorted([e for e in ev if lo <= e[0] < hi], key=lambda e: e[0]):
            f(*a)

        if post:
            tail()
            for c in range(NG - 1):
                o_cp(c).wait()
            for i in range(LASTSUB):
                o_cp(NG - 1, i, LASTSUB).wait()
            return
        assert not lnq and not lnstage
        sh = 0 if pre else NG
        for i, c in enumerate(LIVE_Q):
            q_c[i] = _pk(qs[c + sh].T)
        for i, c in enumerate(LIVE_MX):
            m_c[i] = maccs[c + sh]
        for i, c in enumerate(LIVE_M):
            m_c[len(LIVE_MX) + i] = ms[c + sh]
        for i, c in enumerate(LIVE_O):
            l_c[i] = laccs[c + sh]
        for i, c in enumerate(LIVE_O):
            o_c[i] = oaccs[c + sh]

    zero = zero_ref[0]
    segment(0, 'pre', zero)

    def mid(h, carry):
        segment(h, 'mid', jnp.minimum(h, 0))
        return carry

    lax.fori_loop(0, H - 1, mid, 0)
    segment(H - 1, 'post', zero)


@jax.jit
def pallas_recurrent_scan__mha_block_cached__moe_arch_mod__prompt_kernel(
    A_x: jax.Array,
    A_k_cache: jax.Array,
    A_v_cache: jax.Array,
    A_wq: jax.Array,
    A_wo: jax.Array,
    B_x: jax.Array,
    B_w_r: jax.Array,
    B_w_gate: jax.Array,
    B_w_up: jax.Array,
    B_w_down: jax.Array,
):
    del B_x
    hbm = pl.BlockSpec(memory_space=pl.ANY)
    V = pltpu.VMEM
    dma = pltpu.SemaphoreType.DMA
    out = pl.pallas_call(
        _kernel,
        in_specs=[pl.BlockSpec(memory_space=pltpu.SMEM)] + [hbm] * 9,
        out_specs=hbm,
        out_shape=jax.ShapeDtypeStruct((S, D), bf16),
        scratch_shapes=[
            V((D,), bf16), V((16, D), f32), V((S, D), bf16),
            V((S + 16, DH), bf16), V((S + 16, DH), bf16), V((D + 16, DH), bf16), V((DH + 16, D), bf16),
            V((2 * F + 128, D), bf16), V((2 * NF + 1, D // 2, 128), u32), V((F, D), bf16),
            V((S // 2, D), u32), V((S // 2, D), u32), V((S // 128, 128), f32),
            V((S // 2, DH), u32), V((DH // 2, S), u32), V((D // 2, DH), u32), V((DH // 2, D), u32),
            V((len(LIVE_MX) + len(LIVE_M), 8, G), f32), V((len(LIVE_O), 8, G), f32),
            V((len(LIVE_O), DH, G), f32), V((len(LIVE_Q), DH // 2, G), u32),
            dma((len(XSPLIT),)), dma((4,)), dma((4,)), dma((NG - 1 + LASTSUB,)),
        ] + [V((S, G), f32)] * NSBUF + [V((G // 2, DH), u32)] * NG + [V((G + 16, D), bf16)] * NG
        + [V((G, D), f32)] * NG,
        compiler_params=pltpu.CompilerParams(
            vmem_limit_bytes=100 * 1024 * 1024,
            disable_semaphore_checks=True,
            disable_bounds_checks=True,
        ),
    )(jnp.zeros((1,), jnp.int32), A_x.reshape(S, D), A_k_cache.reshape(H, S, DH), A_v_cache.reshape(H, S, DH),
      A_wq, A_wo, B_w_r, B_w_gate.T, B_w_up.T, B_w_down)
    return out.reshape(1, S, D)
```
